```python
import os as _os
_os.environ.setdefault('JAX_PLATFORMS', 'cpu')
import jax
import jax.numpy as jnp

def _softmax(x, axis=-1):
    return jax.nn.softmax(x, axis=axis)

def _gelu(x):
    return jax.nn.gelu(x, approximate=True)

def _silu(x):
    return jax.nn.silu(x)

def _sigmoid(x):
    return jax.nn.sigmoid(x)

def _layernorm(x, axis=-1, eps=1e-05):
    m = jnp.mean(x, axis=axis, keepdims=True)
    v = jnp.var(x, axis=axis, keepdims=True)
    return (x - m) / jnp.sqrt(v + eps)

def _scatter_add(tgt, idx, src, axis=0):
    return tgt.at[idx].add(src)

def _segment_sum(src, seg, n):
    return jax.ops.segment_sum(src, seg, n)

class _Rng:

    def __init__(self, key):
        self._k = key

    def _next(self):
        self._k, sub = jax.random.split(self._k)
        return sub

    def normal(self, shape):
        return jax.random.normal(self._next(), shape, dtype=jnp.bfloat16)

    def randint(self, lo, hi, shape):
        return jax.random.randint(self._next(), shape, lo, hi, dtype=jnp.int32)

    def uniform(self, shape, lo=0.0, hi=1.0):
        return jax.random.uniform(self._next(), shape, jnp.bfloat16, lo, hi)

    def permutation(self, n):
        return jax.random.permutation(self._next(), n)
kernel_name = 'adaLN_cond__grouped_kv_mqa__swiglu_ffn__prompt'

def setup_inputs():
    _rng = _Rng(jax.random.key(int.from_bytes(__import__("os").urandom(4), "little")))
    _w = lambda a: (lambda t: t.astype(jnp.bfloat16) if jnp.issubdtype(t.dtype, jnp.floating) else t)(jnp.asarray(a))

    def _A_setup():
        B, S, D, H = (1, 2048, 576, 32)
        Dh = D // H
        return {'x': _w((lambda *s: _rng.normal(s) * 0.05)(B, S, D)), 'wq': _w((lambda *s: _rng.normal(s) * 0.05)(D, H * Dh)), 'wk': _w((lambda *s: _rng.normal(s) * 0.05)(D, Dh)), 'wv': _w((lambda *s: _rng.normal(s) * 0.05)(D, Dh)), 'wo': _w((lambda *s: _rng.normal(s) * 0.05)(H * Dh, D))}
    _A_in = _A_setup()

    def _B_setup():
        B, S, D, F = (1, 2048, 576, 4608)
        return {'x': _w((lambda *s: _rng.normal(s) * 0.05)(B, S, D)), 'w_gate': _w((lambda *s: _rng.normal(s) * 0.05)(D, F)), 'w_up': _w((lambda *s: _rng.normal(s) * 0.05)(D, F)), 'w_down': _w((lambda *s: _rng.normal(s) * 0.05)(F, D))}
    _B_in = _B_setup()
    return {'A_x': _A_in['x'], 'A_wq': _A_in['wq'], 'A_wk': _A_in['wk'], 'A_wv': _A_in['wv'], 'A_wo': _A_in['wo'], 'B_x': _B_in['x'], 'B_w_gate': _B_in['w_gate'], 'B_w_up': _B_in['w_up'], 'B_w_down': _B_in['w_down'], 'c': _w((lambda *s: _rng.normal(s) * 0.05)(1, 576) * 8.0), 'w_mod': _w((lambda *s: _rng.normal(s) * 0.05)(576, 6 * 576) * 576 ** (-0.5) * 8.0)}

def reference(A_x, A_wq, A_wk, A_wv, A_wo, B_x, B_w_gate, B_w_up, B_w_down, c, w_mod):

    def _A_ref(x, wq, wk, wv, wo):
        B, S, D = x.shape
        H = 32
        Dh = D // H
        q = (lambda x, *d: x.transpose(*d))((x @ wq).reshape(B, S, H, Dh), 0, 2, 1, 3)
        k = x @ wk
        v = x @ wv
        scores = jnp.einsum('bhqd,bkd->bhqk', q, k) * Dh ** (-0.5)
        p = _softmax(scores, axis=-1)
        o = jnp.einsum('bhqk,bkd->bhqd', p, v)
        return (lambda x, *d: x.transpose(*d))(o, 0, 2, 1, 3).reshape(B, S, H * Dh) @ wo

    def _B_ref(x, w_gate, w_up, w_down):
        g = _silu(x @ w_gate)
        u = x @ w_up
        return g * u @ w_down
    x = A_x
    mod = (_silu(c) @ w_mod).reshape(c.shape[0], 6, 1, -1)
    sa, ca, ga, sb, cb, gb = (mod[:, 0].copy(), mod[:, 1].copy(), mod[:, 2].copy(), mod[:, 3].copy(), mod[:, 4].copy(), mod[:, 5].copy())
    h = _layernorm(x, axis=-1) * (1 + ca) + sa
    x = x + ga * _A_ref(h, A_wq, A_wk, A_wv, A_wo)
    h = _layernorm(x, axis=-1) * (1 + cb) + sb
    x = x + gb * _B_ref(h, B_w_gate, B_w_up, B_w_down)
    return x
```

```python
import functools
import jax
import jax.numpy as jnp
from jax import lax
import jax.experimental.pallas as pl
import jax.experimental.pallas.tpu as pltpu

S, D, H, DH, F = 2048, 576, 32, 18, 4608
TB = 128
NB = S // TB
NC = S // 128
FG = F // 4
NFT = FG // 128
EPS = 1e-5
LOG2E = 1.4426950408889634
QSCALE = DH ** -0.5 * LOG2E
TBOUND = 60.0
f32, bf16, u32, i32 = jnp.float32, jnp.bfloat16, jnp.uint32, jnp.int32
KT = [(0, 128), (128, 128), (256, 128), (384, 128), (512, 64)]
VSLOTS = ([3, 7, 11, 15], [1, 5, 9, 13])
KORDER = tuple([s for s in range(16) if s not in vs] + [vs[0], vs[2], vs[1], vs[3]] for vs in VSLOTS)
NT = (((1,), (1,)), ((), ()))
NIT = 70


def _bf(x):
    return pltpu.bitcast(x, bf16)


def _u32(x):
    return pltpu.bitcast(x.astype(bf16), u32)


def _ln0(x):
    m = jnp.mean(x, axis=0, keepdims=True)
    xc = x - m
    v = jnp.mean(xc * xc, axis=0, keepdims=True)
    return xc * lax.rsqrt(v + EPS)


def _eye(n):
    return (lax.broadcasted_iota(i32, (n, n), 0) == lax.broadcasted_iota(i32, (n, n), 1)).astype(bf16)


def _mm4(w_ref, rhs):
    return jnp.concatenate([jnp.dot(w_ref[r:r + 144, :], rhs, preferred_element_type=f32)
                            for r in range(0, D, 144)], axis=0)


def make(NVF=4, NVA=2, DS=4, PU=4, force_slow=0):
    DR = D // DS

    def kern(c_ref, wkt_ref, wvt_ref, xt_hbm, wq_hbm, wo_hbm, wg_hbm, wu_hbm, wdt_hbm, wmod_hbm,
             out_hbm,
             x_v, h1_v, wmod_v, wq_v, wo_v, wqt_v, wot_v, wkv_v, modc_v, q_v, qf_v, k_v, kb_v, vt_v,
             p_v, ot_v, h2_v, a_v, acc_v, y_v, x1_v, o_v, wg_v, wu_v, wd_v, stat_v,
             sem_x, sem_w, sem_f, sem_o, flag_s):
        def x_copy(b):
            return pltpu.make_async_copy(xt_hbm.at[:, pl.ds(b * TB, TB)], x_v.at[b], sem_x.at[b])
        cp_mod1 = pltpu.make_async_copy(wmod_hbm.at[:, pl.ds(0, 2 * D)], wmod_v.at[:, pl.ds(0, 2 * D)], sem_w.at[0])
        cp_mod2 = pltpu.make_async_copy(wmod_hbm.at[:, pl.ds(2 * D, 4 * D)], wmod_v.at[:, pl.ds(2 * D, 4 * D)], sem_w.at[1])
        cp_wq = pltpu.make_async_copy(wq_hbm, wq_v, sem_w.at[2])
        cp_wo = pltpu.make_async_copy(wo_hbm, wo_v, sem_w.at[3])

        def f_copy(w, g):
            src, dst = ((wg_hbm, wg_v), (wu_hbm, wu_v), (wdt_hbm, wd_v))[w]
            return pltpu.make_async_copy(src.at[:, pl.ds(g * FG, FG)], dst.at[g], sem_f.at[w * 4 + g])

        def o_copy(b, slot):
            return pltpu.make_async_copy(o_v.at[slot], out_hbm.at[:, pl.ds(pl.multiple_of(b * TB, TB), TB)], sem_o.at[slot])

        cp_mod1.start()
        for b in range(NB):
            x_copy(b).start()
        cp_wq.start()

        c = c_ref[...].astype(f32)
        sc = jnp.broadcast_to((c * jax.nn.sigmoid(c)).astype(bf16), (16, D))
        wkv_v[...] = jnp.zeros(wkv_v.shape, bf16)
        wkv_v[0:DH, :] = wkt_ref[...]
        wkv_v[32:32 + DH, :] = wvt_ref[...]

        def mod_cols(c0, n):
            m = jnp.dot(sc, wmod_v[:, c0:c0 + n], preferred_element_type=f32)[0:1]
            return jnp.broadcast_to(m, (128, n)).T

        cp_mod1.wait()
        m1 = mod_cols(0, 2 * D)
        modc_v[0] = m1[0:D]
        modc_v[1] = 1.0 + m1[D:2 * D]

        eye = _eye(128)
        ebig = (lax.broadcasted_iota(i32, (32, DH * 128), 0)
                == lax.shift_right_logical(lax.broadcasted_iota(i32, (32, DH * 128), 1), 7)).astype(bf16)
        row32 = lax.broadcasted_iota(i32, (32, TB), 0)

        def kv_loop(i, carry):
            kn, va = carry
            bs = [i * PU + j for j in range(PU)]
            for b in bs:
                x_copy(b).wait()
            h1s = []
            for b in bs:
                h1 = (_ln0(x_v[b].astype(f32)) * modc_v[1] + modc_v[0]).astype(bf16)
                h1_v[b] = h1
                h1s.append(h1)
            kvts = [jnp.dot(wkv_v[...], h1, preferred_element_type=f32) for h1 in h1s]
            ktoks = []
            for b, kvt in zip(bs, kvts):
                ktb = kvt[0:32].astype(bf16)
                kt = ktb.astype(f32)
                kn = jnp.maximum(kn, jnp.sum(kt * kt, axis=0, keepdims=True))
                va = jnp.maximum(va, jnp.abs(kvt[32:64]))
                lanes = pl.ds(pl.multiple_of(b * TB, TB), TB)
                for v in range(4):
                    vt = kvt[32 - 2 * v:64 - 2 * v]
                    vt = jnp.where(row32 == (0 if v == 3 else 23), 1.0, vt)
                    vt_v[v, :, lanes] = _u32(vt)
                kt128 = jnp.concatenate([ktb, jnp.zeros((96, TB), bf16)], axis=0)
                ktoks.append(lax.dot_general(eye, kt128, NT, preferred_element_type=f32))
            kodds = []
            for b, ktok in zip(bs, ktoks):
                rows = pl.ds(pl.multiple_of(b * 64, 64), 64)
                for par in range(2):
                    ko = jnp.concatenate([ktok[8 * s:8 * s + 8] for s in KORDER[par]], axis=0)
                    ku = _u32(ko)
                    for u in range(par, 8, 2):
                        k_v[u, rows, :] = ku if u == 0 else pltpu.roll(ku, 2 * u, 1)
                kodds += [ktok[8 * s:8 * s + 8, 0:32] for s in range(1, 16, 2)]
            kodd = jnp.concatenate(kodds, axis=0).astype(bf16)
            rows = pl.ds(pl.multiple_of(i * (PU * 64), 64), PU * 64)
            kb_v[rows, :] = jnp.dot(kodd, ebig, preferred_element_type=f32)
            return kn, va

        with jax.named_scope("S_kvloop"):
          kn, va = lax.fori_loop(0, NB // PU, kv_loop, (jnp.zeros((1, TB), f32), jnp.zeros((32, TB), f32)))
        cp_mod2.start()
        cp_wo.start()
        kn2 = jnp.max(kn, axis=1, keepdims=True)
        vrow = jnp.max(va, axis=1, keepdims=True)
        v_ok = jnp.logical_or(vrow == 0.0, jnp.logical_and(vrow >= 2.0 ** -40, vrow <= 2.0 ** 40))
        v_bad = jnp.max(jnp.where(v_ok, 0.0, 1.0), axis=0, keepdims=True)
        lim = jnp.where(v_bad > 0.0, -1.0, TBOUND * TBOUND / 1.02)
        stat_v[0:1, :] = jnp.broadcast_to(kn2, (1, 128))
        stat_v[1:2, :] = jnp.broadcast_to(lim, (1, 128))

        cp_wq.wait()
        wqt_v[...] = wq_v[...].T
        seg = (lax.broadcasted_iota(i32, (H, D), 1) // DH == lax.broadcasted_iota(i32, (H, D), 0)).astype(bf16)

        def q_block(b, slot):
            qt = _mm4(wqt_v, h1_v[b]) * QSCALE
            qb = qt.astype(bf16)
            qr = qb.astype(f32)
            for g in range(4):
                r0 = 144 * g
                q_v[slot * 4 + g, 0:72, :] = pltpu.bitcast(qb[r0:r0 + 144], u32)
                qf_v[slot * 4 + g, 0:72, 0:128] = qr[r0:r0 + 72]
                qf_v[slot * 4 + g, 0:72, 128:256] = qr[r0 + 72:r0 + 144]
            qn = jnp.dot(seg, (qr * qr).astype(bf16), preferred_element_type=f32)
            qn = jnp.max(qn, axis=0, keepdims=True)
            ok = jnp.where(qn * stat_v[0:1, :] <= stat_v[1:2, :], 1.0, 0.0)
            flag_s[slot] = (jnp.min(ok) > 0.5).astype(i32) * (0 if force_slow else 1)

        q_block(0, 0)
        q_block(1, 1)

        def late_setup():
            cp_mod2.wait()
            cp_wo.wait()
            m2 = mod_cols(2 * D, 4 * D)
            modc_v[2] = m2[0:D]
            modc_v[3] = m2[D:2 * D]
            modc_v[4] = 1.0 + m2[2 * D:3 * D]
            modc_v[5] = m2[3 * D:4 * D]
            wot_v[...] = wo_v[...].T

        row24 = lax.broadcasted_iota(i32, (24, TB), 0)

        def body(n, A, B, C, Dn, NV):
            qi = n % 8
            gb = (n + 3) % 4
            gc = (n + 3) % 4
            gd = (n + 2) % 4
            par = n % 2
            RM = 128 - 8 * NV
            o = [None] * 8
            carry = [None]

            def score1(u, c):
                w = 8 * ((DH * u) // 16)
                s = jnp.dot(_bf(k_v[u, c * 64:c * 64 + RM // 2, 0:32]), _bf(q_v[qi, w:w + 16, :]),
                            preferred_element_type=f32)
                order = KORDER[u % 2]
                rows = []
                for slot in range(16):
                    pos = order.index(slot)
                    if pos < 16 - NV:
                        rows.append(s[8 * pos:8 * pos + 8])
                    else:
                        r0 = c * 64 + (slot // 2) * 8
                        lo = (u // 4) * 128
                        sv = None
                        for d in range(DH):
                            qr = DH * (u % 4) + d
                            term = kb_v[r0:r0 + 8, d * 128:(d + 1) * 128] * qf_v[qi, qr:qr + 1, lo:lo + 128]
                            sv = term if sv is None else sv + term
                        rows.append(sv)
                return jnp.concatenate(rows, axis=0)

            def score(up, c):
                sa = jnp.concatenate([score1(2 * up, c), score1(2 * up + 1, c)], axis=1)
                p_v[up, c] = jnp.exp2(sa).astype(bf16)

            def pv(up, c):
                for u in (2 * up, 2 * up + 1):
                    oc = jnp.dot(_bf(vt_v[u % 4, :, c * 128:(c + 1) * 128]),
                                 p_v[up, c, :, (u % 2) * 128:(u % 2 + 1) * 128],
                                 preferred_element_type=f32)[0:24]
                    o[u] = oc if o[u] is None else o[u] + oc
                    if c == NC - 1:
                        r1 = 0 if u % 4 == 3 else 23
                        on = jnp.where(row24 == r1, 0.0, o[u] * (1.0 / o[u][r1:r1 + 1]))
                        base = 16 * u + 8 * (u // 4)
                        first = on[0:8] if u % 4 == 0 else on[0:8] + carry[0]
                        ot_v[gb, base:base + 8, :] = first
                        if u % 4 == 3:
                            ot_v[gb, base + 8:base + 24, :] = on[8:24]
                        else:
                            ot_v[gb, base + 8:base + 16, :] = on[8:16]
                            carry[0] = on[16:24]

            def piece(kind, f, j):
                cols = slice(f * 128, (f + 1) * 128)
                if kind in "gu":
                    w_ref = wg_v if kind == "g" else wu_v
                    ai = 2 * f + (kind == "u")
                    k0, kn_ = KT[j]
                    r = jnp.dot(_bf(h2_v[:, k0:k0 + kn_]), w_ref[gc, k0:k0 + kn_, cols], preferred_element_type=f32)
                    if j > 0:
                        r = r + acc_v[par, ai]
                    if j < 4:
                        acc_v[par, ai] = r
                    elif kind == "g":
                        acc_v[par, ai] = r * pl.reciprocal(1.0 + jnp.exp2(r * (-LOG2E)), approx=True)
                    else:
                        a_v[:, cols] = (acc_v[par, ai - 1] * r).astype(bf16)
                else:
                    yc = lax.dot_general(wd_v[gd, j * DR:(j + 1) * DR, cols], a_v[:, cols], NT,
                                         preferred_element_type=f32)
                    y_v[j * DR:(j + 1) * DR, :] += yc

            gl = []
            if C:
                gl = [(k, f, j) for j in range(4) for f in range(NFT) for k in "gu"]
                gl += [("g", f, 4) for f in range(NFT)] + [("u", f, 4) for f in range(NFT)]
            dl = [("d", f, j) for f in range(NFT) for j in range(DS)] if Dn else []
            fp = []
            di = 0
            for m, gp in enumerate(gl):
                fp.append(gp)
                while di < len(dl) and di * 72 <= m * len(dl):
                    fp.append(dl[di])
                    di += 1
            fp += dl[di:]
            nF = len(fp)
            fi = 0
            atasks = [(up, c) for up in range(4) for c in range(NC)] if (A or B) else []
            nA = len(atasks)
            for idx, t in enumerate(atasks):
                if B:
                    pv(*t)
                while fi < nF and fi * 2 * nA <= (2 * idx) * nF:
                    piece(*fp[fi])
                    fi += 1
                if A:
                    score(*t)
                while fi < nF and fi * 2 * nA <= (2 * idx + 1) * nF:
                    piece(*fp[fi])
                    fi += 1
            while fi < nF:
                piece(*fp[fi])
                fi += 1

        def a_slow(n):
            qi = n % 8

            def pair(up, carry):
                ps = []
                for par in range(2):
                    u = 2 * up + par
                    w = pl.multiple_of(8 * ((DH * u) // 16), 8)
                    s = jnp.dot(_bf(k_v[u, :, 0:32]), _bf(q_v[qi, pl.ds(w, 16), :]), preferred_element_type=f32)
                    p = jnp.exp2(s - jnp.max(s, axis=0, keepdims=True)).reshape(NC, 16, 8, TB)
                    order = KORDER[par]
                    p = jnp.concatenate([p[:, order.index(sl):order.index(sl) + 1] for sl in range(16)], axis=1)
                    ps.append(p.reshape(NC, 128, TB))
                p_v[up] = jnp.concatenate(ps, axis=2).astype(bf16)
                return carry

            lax.fori_loop(0, 4, pair, 0)

        def e1(b):
            ot = jnp.concatenate([ot_v[g, 0:144, :] for g in range(4)], axis=0).astype(bf16)
            att = _mm4(wot_v, ot)
            x1 = x_v[b].astype(f32) + modc_v[2] * att
            x1_v[b % 2] = x1
            q_block(jnp.minimum(b + 2, NB - 1), b % 2)
            h2t = (_ln0(x1) * modc_v[4] + modc_v[3]).astype(bf16)
            h2 = lax.dot_general(_eye(128), h2t, NT, preferred_element_type=f32)
            h2_v[:, 0:D] = _u32(h2)

        def e2(b):
            slot = b % 2

            @pl.when(b >= 2)
            def _():
                o_copy(b - 2, slot).wait()

            o_v[slot] = (x1_v[slot] + modc_v[5] * y_v[...]).astype(bf16)
            o_copy(b, slot).start()

        def step(n, carry):
            fast = jnp.logical_and(n < 64, flag_s[(n // 4) % 2] == 1)
            fused = jnp.logical_and(fast, n >= 5)

            for g in range(4):
              @pl.when(n == g)
              def _():
                for w in range(3):
                    f_copy(w, g).start()

            with jax.named_scope("S_late"):
              @pl.when(n == 2)
              def _():
                late_setup()

            with jax.named_scope("S_wait"):
              @pl.when(jnp.logical_and(n >= 5, n <= 8))
              def _():
                g = n - 5
                for w in range(3):
                    src, dst = ((wg_hbm, wg_v), (wu_hbm, wu_v), (wdt_hbm, wd_v))[w]
                    pltpu.make_async_copy(src.at[:, pl.ds(0, FG)], dst.at[g], sem_f.at[w * 4 + g]).wait()

            with jax.named_scope("S_fused"):
              @pl.when(jnp.logical_and(fused, n >= 6))
              def _():
                body(n, 1, 1, 1, 1, NVF)

            with jax.named_scope("S_ab"):
              @pl.when(jnp.logical_and(fast, n <= 5))
              def _():
                body(n, 1, 1, 0, 0, NVA)

            with jax.named_scope("S_tail"):
              @pl.when(jnp.logical_not(fast))
              def _():
                @pl.when(jnp.logical_and(n >= 1, n <= 64))
                def _():
                    body(n, 0, 1, 0, 0, 0)

                @pl.when(n < 64)
                def _():
                    a_slow(n)

                @pl.when(jnp.logical_and(n >= 6, n <= 68))
                def _():
                    body(n, 0, 0, 1, 1, 0)

                @pl.when(n == 69)
                def _():
                    body(n, 0, 0, 0, 1, 0)

            with jax.named_scope("S_c5"):
              @pl.when(n == 5)
              def _():
                body(n, 0, 0, 1, 0, 0)
                y_v[...] = jnp.zeros(y_v.shape, f32)

            with jax.named_scope("S_e1"):
              @pl.when(jnp.logical_and(n % 4 == 0, jnp.logical_and(n >= 4, n <= 64)))
              def _():
                e1(n // 4 - 1)

            with jax.named_scope("S_e2"):
              @pl.when(jnp.logical_and(n % 4 == 1, n >= 9))
              def _():
                e2((n - 9) // 4)
                y_v[...] = jnp.zeros(y_v.shape, f32)

            return carry

        with jax.named_scope("S_main"):
          lax.fori_loop(0, NIT, step, 0)
        o_copy(NB - 2, 0).wait()
        o_copy(NB - 1, 1).wait()

    def call(A_x, A_wq, A_wk, A_wv, A_wo, B_x, B_w_gate, B_w_up, B_w_down, c, w_mod):
        xt = A_x.reshape(S, D).T
        vm = pl.BlockSpec(memory_space=pltpu.VMEM)
        hb = pl.BlockSpec(memory_space=pl.ANY)
        out = pl.pallas_call(
            kern,
            in_specs=[vm, vm, vm, hb, hb, hb, hb, hb, hb, hb],
            out_specs=hb,
            out_shape=jax.ShapeDtypeStruct((D, S), bf16),
            scratch_shapes=[
                pltpu.VMEM((NB, D, TB), bf16),
                pltpu.VMEM((NB, D, TB), bf16),
                pltpu.VMEM((D, 6 * D), bf16),
                pltpu.VMEM((D, D), bf16),
                pltpu.VMEM((D, D), bf16),
                pltpu.VMEM((D, D), bf16),
                pltpu.VMEM((D, D), bf16),
                pltpu.VMEM((64, D), bf16),
                pltpu.VMEM((6, D, 128), f32),
                pltpu.VMEM((8, 96, 128), u32),
                pltpu.VMEM((8, 80, 256), f32),
                pltpu.VMEM((8, S // 2, 128), u32),
                pltpu.VMEM((S // 2, DH * 128), f32),
                pltpu.VMEM((4, 16, S), u32),
                pltpu.VMEM((4, NC, 128, 256), bf16),
                pltpu.VMEM((4, 160, TB), f32),
                pltpu.VMEM((64, 640), u32),
                pltpu.VMEM((TB, 1280), bf16),
                pltpu.VMEM((2, 2 * NFT, TB, 128), f32),
                pltpu.VMEM((D, TB), f32),
                pltpu.VMEM((2, D, TB), f32),
                pltpu.VMEM((2, D, TB), bf16),
                pltpu.VMEM((4, D, FG), bf16),
                pltpu.VMEM((4, D, FG), bf16),
                pltpu.VMEM((4, D, FG), bf16),
                pltpu.VMEM((32, 128), f32),
                pltpu.SemaphoreType.DMA((NB,)),
                pltpu.SemaphoreType.DMA((4,)),
                pltpu.SemaphoreType.DMA((12,)),
                pltpu.SemaphoreType.DMA((2,)),
                pltpu.SMEM((2,), i32),
            ],
            compiler_params=pltpu.CompilerParams(vmem_limit_bytes=110 * 1024 * 1024),
            name="v3k",
        )(c, A_wk.T, A_wv.T, xt, A_wq, A_wo, B_w_gate, B_w_up, B_w_down.T, w_mod)
        return out.T.reshape(1, S, D)

    return call


_call = make()


@jax.jit
def pallas_adaLN_cond__grouped_kv_mqa__swiglu_ffn__prompt_kernel(A_x, A_wq, A_wk, A_wv, A_wo, B_x, B_w_gate, B_w_up, B_w_down, c, w_mod):
    return _call(A_x, A_wq, A_wk, A_wv, A_wo, B_x, B_w_gate, B_w_up, B_w_down, c, w_mod)
```

```python
import functools

import jax
import jax.numpy as jnp
from jax import lax
import jax.experimental.pallas as pl
import jax.experimental.pallas.tpu as pltpu

S, D, H, DH, F = 2048, 576, 32, 18, 4608
TB = 128
NB = S // TB
NCP = S // 256
FG = F // 4
NFT = FG // 128
EPS = 1e-5
LOG2E = 1.4426950408889634
QSCALE = DH ** -0.5 * LOG2E
TBOUND = 60.0
f32, bf16, u32, i32 = jnp.float32, jnp.bfloat16, jnp.uint32, jnp.int32
KT = [(0, 128), (128, 128), (256, 128), (384, 128), (512, 64)]
VSLOTS = {8: [0, 3, 6, 9, 2, 5, 8, 11], 10: [0, 4, 8, 12, 1, 5, 9, 3, 7, 11]}
KORDER = {nv: [(sl, hf) for sl in range(16) for hf in range(2) if not (hf == 1 and sl in vs)] + [(sl, 1) for sl in vs]
          for nv, vs in VSLOTS.items()}
DRS = [(0, 128), (128, 256), (256, 384), (384, 512), (512, 576)]
NT = (((1,), (1,)), ((), ()))
DEBUG = False


def _bf(x):
    return pltpu.bitcast(x, bf16)


def _u32(x):
    return pltpu.bitcast(x.astype(bf16), u32)


def _stats_part(x, piv):
    d = (x - piv).reshape(x.shape[0] // 8, 8, TB)
    return jnp.sum(d, axis=0), jnp.sum(d * d, axis=0)


def _stats_fin(parts, piv):
    s1 = sum(p[0] for p in parts[1:]) + parts[0][0]
    s2 = sum(p[1] for p in parts[1:]) + parts[0][1]
    m1 = jnp.sum(s1, axis=0, keepdims=True) * (1.0 / D)
    m2 = jnp.sum(s2, axis=0, keepdims=True) * (1.0 / D)
    var = jnp.maximum(m2 - m1 * m1, 0.0)
    return piv + m1, lax.rsqrt(var + EPS)


def _stats(x):
    piv = x[0:1]
    return _stats_fin([_stats_part(x[r:r + 144], piv) for r in range(0, D, 144)], piv)


def _eye(n):
    return (lax.broadcasted_iota(i32, (n, n), 0) == lax.broadcasted_iota(i32, (n, n), 1)).astype(bf16)


def _mm4(w_ref, rhs):
    return jnp.concatenate([jnp.dot(w_ref[r:r + 144, :], rhs, preferred_element_type=f32)
                            for r in range(0, D, 144)], axis=0)


def _unorder(s, nv):
    halves = []
    for hf in range(2):
        runs = []
        for sl in range(16):
            pos = KORDER[nv].index((sl, hf))
            if runs and runs[-1][1] == pos:
                runs[-1][1] = pos + 1
            else:
                runs.append([pos, pos + 1])
        halves.append(jnp.concatenate([s[8 * a:8 * b] for a, b in runs], axis=0))
    return jnp.concatenate(halves, axis=1)


def make(NVA=4, force_slow=0, E1POS=3, FRONT=6, TREE=2, M10=0xEE, TOL=-192, NX=0, TIN=0, HB=2, HA=2, NVH=8, NE=4, NVE=6, WOF=0, DW=1, NVW=8, NVW4=6, T0=64, only_super=0, NL=2, NVL=4, WQ=12, QP=16, XWM=0):
    XW = [{0: 4, 4: 8, 8: 12, 12: 16}, {0: 2, 2: 4, 4: 8, 8: 16}, {0: 4, 4: 8, 8: 16}][XWM]
    FSTART = {0: [(0, 0), (1, 0)], 1: [(2, 0), (0, 1), (1, 1)], 2: [(2, 1), (0, 2), (1, 2)],
              3: [(2, 2), (0, 3), (1, 3), (2, 3)]}
    FWAIT = {6: [(0, 0), (1, 0)], 7: [(2, 0), (0, 1), (1, 1)]}
    LATE = 3
    NVC = [10 if (M10 >> c) & 1 else 8 for c in range(NCP)]
    KBE = [8 * sum(NVC[:c + 1]) for c in range(NCP)]

    def kern(c_hbm, wkt_hbm, wvt_hbm, xt_hbm, wq_hbm, wo_hbm, wg_hbm, wu_hbm, wdt_hbm, wmod_hbm,
             out_hbm,
             x_v, wmod_v, wq_v, wo_v, wqt_v, wot_v, wkv_v, modc_v, q_v, qf_v, k_v, kb_v, vt_v,
             p_v, ot_v, h2_v, h2n_v, h2t_v, ln_v, a_v, acc_v, y_v, x1_v, o_v, wg_v, wu_v, wd_v, stat_v, c_ref, wkt_ref, wvt_ref,
             sem_x, sem_w, sem_f, sem_o, flag_s):
        def x_copy(b):
            return pltpu.make_async_copy(xt_hbm.at[:, pl.ds(b * TB, TB)], x_v.at[b], sem_x.at[b])

        cp_mod1 = pltpu.make_async_copy(wmod_hbm.at[:, pl.ds(0, 2 * D)], wmod_v.at[:, pl.ds(0, 2 * D)], sem_w.at[6])

        def wq_copy(j):
            return pltpu.make_async_copy(wq_hbm.at[pl.ds(j * 144, 144), :], wq_v.at[pl.ds(j * 144, 144), :],
                                         sem_w.at[2 + j])

        cp_mod2 = pltpu.make_async_copy(wmod_hbm.at[:, pl.ds(2 * D, 4 * D)], wmod_v.at[:, pl.ds(2 * D, 4 * D)], sem_w.at[0])
        cp_wo = pltpu.make_async_copy(wo_hbm, wo_v, sem_w.at[1])

        def f_copy(w, g):
            src, dst = ((wg_hbm, wg_v), (wu_hbm, wu_v), (wdt_hbm, wd_v))[w]
            return pltpu.make_async_copy(src.at[:, pl.ds(g * FG, FG)], dst.at[g], sem_f.at[w * 4 + g])

        def o_copy(b, slot):
            return pltpu.make_async_copy(o_v.at[slot], out_hbm.at[:, pl.ds(pl.multiple_of(b * TB, TB), TB)], sem_o.at[slot])

        small = [pltpu.make_async_copy(src, dst, sem_w.at[7 + i]) for i, (src, dst) in enumerate(
            [(c_hbm, c_ref), (wkt_hbm, wkt_ref), (wvt_hbm, wvt_ref)])]
        for cp in small:
            cp.start()
        cp_mod1.start()
        for cp in small:
            cp.wait()

        c = c_ref[...].astype(f32)
        sc = jnp.broadcast_to((c * jax.nn.sigmoid(c)).astype(bf16), (16, D))
        wkv_v[...] = jnp.zeros(wkv_v.shape, bf16)
        wkv_v[0:DH, :] = wkt_ref[...]
        wkv_v[32:32 + DH, :] = wvt_ref[...]

        def mod_cols(c0, n):
            m = jnp.dot(sc, wmod_v[:, c0:c0 + n], preferred_element_type=f32)[0:1]
            return jnp.broadcast_to(m, (128, n)).T

        with jax.named_scope("P_mod"):
            cp_mod1.wait()
            for b in range(NB):
                x_copy(b).start()
            for j in range(4):
                wq_copy(j).start()
            m1 = mod_cols(0, 2 * D)
            modc_v[0] = m1[0:D]
            modc_v[1] = 1.0 + m1[D:2 * D]

        def ln1_stats(b):
            m, r = _stats(x_v[b].astype(f32))
            ln_v[b, 0:1, 0:128] = m
            ln_v[b, 1:2, 0:128] = r

        def h1_of(b):
            xn = (x_v[b].astype(f32) - ln_v[b, 0:1, 0:128]) * ln_v[b, 1:2, 0:128]
            return (xn * modc_v[1] + modc_v[0]).astype(bf16)

        def kv_s1(b):
            ln1_stats(b)
            return jnp.dot(wkv_v[...], h1_of(b), preferred_element_type=f32)

        def kv_s2(b, kvt, kn, va):
            row32 = lax.broadcasted_iota(i32, (32, TB), 0)
            ktb = kvt[0:32].astype(bf16)
            kt = ktb.astype(f32)
            kn = jnp.maximum(kn, jnp.sum(kt * kt, axis=0, keepdims=True))
            va = jnp.maximum(va, jnp.abs(kvt[32:64]))
            for v in range(4):
                vt = kvt[32 - 2 * v:64 - 2 * v]
                vt = jnp.where(row32 == (0 if v == 3 else 23), 1.0, vt)
                vt_v[v, :, b * TB:(b + 1) * TB] = _u32(vt)
            return lax.dot_general(_eye(128), ktb, NT, preferred_element_type=f32), kn, va

        def kv_s3(cp, pair):
            k_v[cp * 128:(cp + 1) * 128, :] = _u32(
                jnp.concatenate([pair[hf][8 * sl:8 * sl + 8] for sl, hf in KORDER[NVC[cp]]], axis=0))

        def kv_s4(cp, half):
            c0, c1 = half * 9 * 128, (half + 1) * 9 * 128
            esel = (lax.broadcasted_iota(i32, (32, 9 * 128), 0)
                    == lax.shift_right_logical(lax.broadcasted_iota(i32, (32, 9 * 128), 1), 7) + 9 * half).astype(bf16)
            kv = _bf(k_v[(cp + 1) * 128 - 4 * NVC[cp]:(cp + 1) * 128, :])
            kb_v[KBE[cp] - 8 * NVC[cp]:KBE[cp], c0:c1] = jnp.dot(kv, esel, preferred_element_type=f32)

        def q_block(h1, slot):
            qt = _mm4(wqt_v, h1) * QSCALE
            qr = qt.astype(bf16).astype(f32)
            z8 = jnp.zeros((8, TB), f32)
            qz = jnp.concatenate([qr, z8], axis=0)
            row8 = lax.broadcasted_iota(i32, (8, TB), 0)
            qn = None
            for g in range(4):
                r0 = 144 * g
                wins = []
                for u in range(8):
                    w = qz[r0 + DH * u:r0 + DH * u + 24]
                    wins += [w, z8]
                    sq = w * w
                    t = sq[0:8] + sq[8:16] + jnp.where(row8 < DH - 16, sq[16:24], 0.0)
                    t = jnp.sum(t, axis=0, keepdims=True)
                    qn = t if qn is None else jnp.maximum(qn, t)
                q_v[slot * 4 + g] = _u32(jnp.concatenate(wins, axis=0))
                qf_v[slot * 4 + g, 0:72, 0:128] = qr[r0:r0 + 72]
                qf_v[slot * 4 + g, 0:72, 128:256] = qr[r0 + 72:r0 + 144]
            return qn

        def set_flag(qn, slot):
            ok = jnp.where(qn * stat_v[0:1, :] <= stat_v[1:2, :], 1.0, 0.0)
            flag_s[slot] = (jnp.min(ok) > 0.5).astype(i32) * (0 if force_slow else 1)

        kn = jnp.zeros((1, TB), f32)
        va = jnp.zeros((32, TB), f32)
        kvts, ktoks = {}, {}
        with jax.named_scope("P_kv"):
            for i in range(NB + 5):
                if i in XW:
                    for b in range(i, XW[i]):
                        x_copy(b).wait()
                if i == WQ:
                    for j in range(4):
                        wq_copy(j).wait()
                    cp_mod2.start()
                    cp_wo.start()
                    wqt_v[...] = wq_v[...].T
                if i < NB:
                    kvts[i] = kv_s1(i)
                if 0 <= i - 1 < NB:
                    ktoks[i - 1], kn, va = kv_s2(i - 1, kvts.pop(i - 1), kn, va)
                if i == QP:
                    qn0 = q_block(h1_of(0), 0)
                if i >= 3 and i % 2 == 1 and (i - 3) // 2 < NCP:
                    cp = (i - 3) // 2
                    kv_s3(cp, [ktoks.pop(2 * cp), ktoks.pop(2 * cp + 1)])
                if i >= 3 and (i - 3) // 2 < NCP:
                    kv_s4((i - 3) // 2, (i - 3) % 2)
            kn2 = jnp.max(kn, axis=1, keepdims=True)
            vrow = jnp.max(va, axis=1, keepdims=True)
            v_ok = jnp.logical_or(vrow == 0.0, jnp.logical_and(vrow >= 2.0 ** -40, vrow <= 2.0 ** 40))
            v_bad = jnp.max(jnp.where(v_ok, 0.0, 1.0), axis=0, keepdims=True)
            lim = jnp.where(v_bad > 0.0, -1.0, TBOUND * TBOUND / 1.02)
            stat_v[0:1, :] = jnp.broadcast_to(kn2, (1, 128))
            stat_v[1:2, :] = jnp.broadcast_to(lim, (1, 128))
            set_flag(qn0, 0)

        def late_setup():
            cp_mod2.wait()
            cp_wo.wait()
            set_flag(q_block(h1_of(1), 1), 1)
            m2 = mod_cols(2 * D, 4 * D)
            modc_v[2] = m2[0:D]
            modc_v[3] = m2[D:2 * D]
            modc_v[4] = 1.0 + m2[2 * D:3 * D]
            modc_v[5] = m2[3 * D:4 * D]
            wot_v[...] = wo_v[...].T

        class Unit:
            def __init__(self, qi, gb, gc, gd, par, NV, y_first=False):
                self.qi, self.gb, self.gc, self.gd, self.par, self.NV = qi, gb, gc, gd, par, NV
                self.y_first = y_first
                self.o = [None] * 8
                self.carry = None
                self.qrows = {}
                self.nvt = {}

            def score_a(self, u, c):
                return jnp.dot(_bf(k_v[c * 128:c * 128 + 64, :]), _bf(q_v[self.qi, 16 * u:16 * u + 16, :]),
                               preferred_element_type=f32)

            def nv(self, u, c):
                return self.nvt[(u, c)] if self.NV is None else self.NV

            def score_b(self, u, c):
                return jnp.dot(_bf(k_v[c * 128 + 64:(c + 1) * 128 - 4 * self.nv(u, c), :]),
                               _bf(q_v[self.qi, 16 * u:16 * u + 16, :]), preferred_element_type=f32)

            def score_end(self, u, c, sa, sb):
                NV = self.nv(u, c)
                if u not in self.qrows:
                    lo = (u // 4) * 128
                    q0 = DH * (u % 4)
                    self.qrows[u] = jnp.concatenate(
                        [jnp.broadcast_to(qf_v[self.qi, q0 + d:q0 + d + 1, lo:lo + 128], (8, TB)) for d in range(DH)],
                        axis=1)[None]
                prod = kb_v[KBE[c] - 8 * NV:KBE[c], :].reshape(NV, 8, DH * 128) * self.qrows[u]
                w = TREE * 128
                sv = prod[:, :, 0:w]
                for d in range(1, DH // TREE):
                    sv = sv + prod[:, :, d * w:(d + 1) * w]
                s1 = sv[:, :, 0:128]
                for d in range(1, TREE):
                    s1 = s1 + sv[:, :, d * 128:(d + 1) * 128]
                s = jnp.concatenate([sa, sb, s1.reshape(8 * NV, TB)], axis=0)
                p_v[u, c] = jnp.exp2(_unorder(s, NVC[c])).astype(bf16)

            def pv(self, u, c, hf):
                o = self.o
                k0 = c * 256 + hf * 128
                oc = jnp.dot(_bf(vt_v[u % 4, :, k0:k0 + 128]), p_v[u, c, :, hf * 128:(hf + 1) * 128],
                             preferred_element_type=f32)[0:24]
                o[u] = oc if o[u] is None else o[u] + oc
                if c == NCP - 1 and hf == 1:
                    row24 = lax.broadcasted_iota(i32, (24, TB), 0)
                    r1 = 0 if u % 4 == 3 else 23
                    on = jnp.where(row24 == r1, 0.0, o[u] * (1.0 / o[u][r1:r1 + 1]))
                    base = 16 * u + 8 * (u // 4)
                    first = on[0:8] if u % 4 == 0 else on[0:8] + self.carry
                    ot_v[self.gb, base:base + 8, :] = first
                    if u % 4 == 3:
                        ot_v[self.gb, base + 8:base + 24, :] = on[8:24]
                    else:
                        ot_v[self.gb, base + 8:base + 16, :] = on[8:16]
                        self.carry = on[16:24]

            def piece(self, kind, f, j):
                cols = slice(f * 128, (f + 1) * 128)
                par = self.par
                if kind in "gu":
                    w_ref = wg_v if kind == "g" else wu_v
                    ai = 2 * f + (kind == "u")
                    k0, kn_ = KT[j]
                    r = jnp.dot(_bf(h2_v[:, k0:k0 + kn_]), w_ref[self.gc, k0:k0 + kn_, cols],
                                preferred_element_type=f32)
                    if j > 0:
                        r = r + acc_v[par, ai]
                    if j < 4:
                        acc_v[par, ai] = r
                    elif kind == "g":
                        acc_v[par, ai] = r * pl.reciprocal(1.0 + jnp.exp2(r * (-LOG2E)), approx=True)
                    else:
                        a_v[:, cols] = (acc_v[par, ai - 1] * r).astype(bf16)
                else:
                    ra, rb = DRS[j]
                    yc = lax.dot_general(wd_v[self.gd, ra:rb, cols], a_v[:, cols], NT, preferred_element_type=f32)
                    if self.y_first and f == 0:
                        y_v[ra:rb, :] = yc
                    else:
                        y_v[ra:rb, :] += yc

            def ffn_list(self, C, Dn, front=0, flip=0):
                gl = []
                if C:
                    gl = [(k, f, j) for j in range(4) for f in range(NFT) for k in "gu"]
                    for i in range(NFT + 1):
                        gl += ([("g", i, 4)] if i < NFT else []) + ([("u", i - 1, 4)] if i >= 1 else [])
                dl = []
                if Dn:
                    dl = [("d", f, j) for f in range(NFT)
                          for j in (range(5) if (f + flip) % 2 == 0 else range(4, -1, -1))]
                fp = dl[:front]
                di = front
                for m, gp in enumerate(gl):
                    fp.append(gp)
                    while di < len(dl) and ((di - front) * 72 <= m * (len(dl) - front)
                                            or (di > 0 and dl[di][2] == 4 and dl[di - 1][2] == 4)):
                        fp.append(dl[di])
                        di += 1
                fp += dl[di:]
                return [(DRS[p[2]][1] - DRS[p[2]][0] if p[0] == "d" else 128,
                         functools.partial(self.piece, *p), p) for p in fp]

        ATASKS = [(u, c) for u in range(8) for c in range(NCP)]

        def body(n, A, B, C, Dn, NV):
            un = Unit(n % 8, (n + 3) % 4, (n + 2) % 4, (n + 1) % 4, n % 2, NV)
            for t in (ATASKS if (A or B) else []):
                if B:
                    un.pv(*t, 0)
                    un.pv(*t, 1)
                if A:
                    un.score_end(*t, un.score_a(*t), un.score_b(*t))
            for _, thunk, _ in un.ffn_list(C, Dn):
                thunk()

        def e1_wo(b):
            ot = jnp.concatenate([ot_v[g, 0:144, :] for g in range(4)], axis=0).astype(bf16)
            att = _mm4(wot_v, ot)
            x1 = x_v[b].astype(f32) + modc_v[2] * att
            x1_v[b % 2] = x1
            return _stats(x1)

        def e1_wo_piece(b, r, j, st):
            k0, kn_ = KT[j]
            segs = []
            for g in range(4):
                lo, hi = max(k0, 144 * g), min(k0 + kn_, 144 * g + 144)
                if lo < hi:
                    segs.append(ot_v[g, lo - 144 * g:hi - 144 * g, :])
            ot = jnp.concatenate(segs, axis=0).astype(bf16)
            rows = slice(144 * r, 144 * r + 144)
            res = jnp.dot(wot_v[rows, k0:k0 + kn_], ot, preferred_element_type=f32)
            if j > 0:
                res = res + x1_v[b % 2, rows, :]
            if j == 4:
                res = x_v[b, rows, :].astype(f32) + modc_v[2, rows, :] * res
                if r == 0:
                    st["piv"] = res[0:1]
                st.setdefault("parts", []).append(_stats_part(res, st["piv"]))
            x1_v[b % 2, rows, :] = res

        def e1_q(b, m, r):
            qn = q_block(h1_of(jnp.minimum(b + 2, NB - 1)), b % 2)
            h2t_v[b % 2] = ((x1_v[b % 2] - m) * r * modc_v[4] + modc_v[3]).astype(bf16)
            return qn

        def e1_core(b):
            return e1_q(b, *e1_wo(b))

        def e1_tr(b, j):
            k0, kn_ = KT[j]
            h2 = lax.dot_general(_eye(128), h2t_v[b % 2, k0:k0 + kn_, :], NT, preferred_element_type=f32)
            h2n_v[b % 2, :, k0:k0 + kn_] = _u32(h2)

        def h2_switch(b, j):
            k0, kn_ = KT[j]
            h2_v[:, k0:k0 + kn_] = h2n_v[b % 2, :, k0:k0 + kn_]

        def e2_core(b):
            o_v[b % 2] = (x1_v[b % 2] + modc_v[5] * y_v[...]).astype(bf16)

        def superbody(B):
            qb = (B % 2) * 4
            units = [Unit(qb + g, (g + 3) % 4, (g + 2) % 4, (g + 1) % 4, B % 2, None, y_first=(g == 3))
                     for g in range(4)]
            l1 = units[1].ffn_list(1, 1)
            for j in range(5):
                i = max(k for k, e in enumerate(l1) if e[2][0] in "gu" and e[2][2] == j)
                l1.insert(i + 1, (0, functools.partial(h2_switch, B - 1, j), ("e", 0, 0)))
            l2 = units[2].ffn_list(1, 1)
            last_d = max(i for i, e in enumerate(l2) if e[2][0] == "d")
            l2.insert(last_d + 1, (0, functools.partial(e2_core, B - 2), ("e", 0, 0)))
            fl = units[0].ffn_list(1, 1) + l1 + l2 + units[3].ffn_list(1, 1)
            hist = []
            tasks = [(un, u, c) for un in units for u, c in ATASKS]
            nt = len(tasks)
            col1 = []
            for t in range(nt + 1):
                if t > 0:
                    col1.append(("b", t - 1))
                if t < nt:
                    col1 += [("p", t, 0), ("p", t, 1)]
            col1 = col1[0:2] + col1[2:]
            sa, sb = {}, {}
            pdone = [False] * nt
            fin = [0]

            def finish():
                while fin[0] < nt and fin[0] in sa and fin[0] in sb and pdone[fin[0]]:
                    un, u, c = tasks[fin[0]]
                    un.score_end(u, c, sa.pop(fin[0]), sb.pop(fin[0]))
                    fin[0] += 1

            def take_f():
                rows, thunk, p = fl.pop(0)
                hist.append(p)
                thunk()
                while fl and fl[0][0] == 0:
                    fl.pop(0)[1]()
                return rows

            T = [T0, 0, T0, T0]
            i0 = 0
            qn = None
            wo_at = 64 + E1POS
            e1_at = 10 ** 6 if WOF else wo_at
            wst = {}
            xleft = NX
            while i0 < nt or col1 or fl:
                k = min((0, 2, 3, 1), key=lambda m: T[m])
                if WOF and i0 == wo_at and not wst:
                    wst["on"] = True
                    for i, (j, r) in enumerate((j, r) for j in range(5) for r in range(4)):
                        fl.insert(i, (144, functools.partial(e1_wo_piece, B - 1, r, j, wst), ("w", r, j)))
                if WOF and e1_at > nt and len(wst.get("parts", ())) == 4:
                    e1_at = i0 + DW
                if qn is None and i0 == e1_at and k == 0:
                    if WOF:
                        qn = e1_q(B - 1, *_stats_fin(wst["parts"], wst["piv"]))
                    else:
                        qn = e1_core(B - 1)
                    for j in range(5):
                        if j < TIN:
                            e1_tr(B - 1, j)
                        else:
                            fl.insert(j - TIN, (128, functools.partial(e1_tr, B - 1, j), ("t", 0, j)))
                    set_flag(qn, (B - 1) % 2)
                    for rows in [144] * (20 if WOF else 40) + [128] * TIN:
                        T[min((0, 2, 3, 1), key=lambda m: T[m])] += rows
                    continue
                if k == 0 and qn is not None and xleft and fl:
                    T[0] += take_f()
                    xleft -= 1
                elif k == 0 and i0 < nt:
                    un, u, c = tasks[i0]
                    sa[i0] = un.score_a(u, c)
                    i0 += 1
                    T[0] += 128
                elif k == 1 and col1:
                    it = col1[0]
                    due = T[0] + 128 * (it[1] - i0) - (64 if it[0] == "p" and it[2] == 0 else 0)
                    lead = due - T[1]
                    blocked = qn is None and it[1] > e1_at
                    if fl and (blocked or (it[0] != "p" or it[2] == 0) and lead + TOL >= fl[0][0]):
                        T[1] += take_f()
                    else:
                        col1.pop(0)
                        un, u, c = tasks[it[1]]
                        if it[0] == "p":
                            if WOF and it[1] >= 64 and c == NCP - 1:
                                lim = 144 * ((it[1] - 64) // 64) + DH * (u + 1) + 8
                                assert not any(e[2][0] == "w" and KT[e[2][2]][0] < lim for e in fl), "ot hazard"
                                assert wst
                            un.pv(u, c, it[2])
                            pdone[it[1]] = it[2] == 1
                            T[1] += 32
                        else:
                            near = hist[-HB:] + [e[2] for e in fl[:HA]]
                            hot = any(p[0] == "g" and p[2] == 4 for p in near)
                            nv = NVC[c]
                            if hot:
                                nv = min(nv, NVH)
                            if any(p[0] == "w" for p in near):
                                nv = min(nv, NVW4 if any(p[0] == "w" and p[2] == 4 for p in near) else NVW)
                            if e1_at <= it[1] < e1_at + NE:
                                nv = min(nv, NVE)
                            if it[1] >= nt - NL:
                                nv = min(nv, NVL)
                            un.nvt[(u, c)] = nv
                            sb[it[1]] = un.score_b(u, c)
                            T[1] += 128 - 8 * nv
                elif fl:
                    T[k] += take_f()
                else:
                    if DEBUG:
                        print("col", k, "ends", T[k], "i0", i0, len(col1))
                    T[k] = 10 ** 9
                finish()

        def a_slow(n):
            qi = n % 8

            def head(u, carry):
                w = pl.multiple_of(16 * u, 16)
                s = jnp.dot(_bf(k_v[...]), _bf(q_v[qi, pl.ds(w, 16), :]), preferred_element_type=f32)
                p = jnp.exp2(s - jnp.max(s, axis=0, keepdims=True))
                for c in range(NCP):
                    p_v[u, c] = _unorder(p[c * 256:(c + 1) * 256], NVC[c]).astype(bf16)
                return carry

            lax.fori_loop(0, 8, head, 0)

        def o_wait(b):
            @pl.when(b >= 2)
            def _():
                o_copy(b - 2, b % 2).wait()

        def step(n, fast):
            with jax.named_scope("S_early"):
                @pl.when(n <= 8)
                def _():
                    for m, starts in FSTART.items():
                        @pl.when(n == m)
                        def _():
                            for w, g in starts:
                                f_copy(w, g).start()

                    @pl.when(n == LATE)
                    def _():
                        late_setup()

                    for m, waits in FWAIT.items():
                        @pl.when(n == m)
                        def _():
                            for w, g in waits:
                                f_copy(w, g).wait()

            with jax.named_scope("S_att"):
                @pl.when(fast)
                def _():
                    body(n, 1, 1, 0, 0, NVA)

                @pl.when(jnp.logical_not(fast))
                def _():
                    @pl.when(jnp.logical_and(n >= 1, n <= 64))
                    def _():
                        body(n, 0, 1, 0, 0, 0)

                    @pl.when(n < 64)
                    def _():
                        a_slow(n)

            with jax.named_scope("S_ffn"):
                @pl.when(jnp.logical_and(n >= 7, n <= 69))
                def _():
                    body(n, 0, 0, 1, 1, 0)

                @pl.when(n == 70)
                def _():
                    body(n, 0, 0, 0, 1, 0)

                @pl.when(n == 6)
                def _():
                    body(n, 0, 0, 1, 0, 0)
                    y_v[...] = jnp.zeros(y_v.shape, f32)

            with jax.named_scope("S_e1"):
                @pl.when(jnp.logical_and(n % 4 == 0, jnp.logical_and(n >= 4, n <= 64)))
                def _():
                    b = n // 4 - 1
                    set_flag(e1_core(b), b % 2)
                    for j in range(5):
                        e1_tr(b, j)

                @pl.when(jnp.logical_and(n % 4 == 1, jnp.logical_and(n >= 5, n <= 65)))
                def _():
                    for j in range(5):
                        h2_switch(n // 4 - 1, j)

            with jax.named_scope("S_e2"):
                @pl.when(jnp.logical_and(n % 4 == 2, n >= 10))
                def _():
                    e2_core(n // 4 - 2)
                    y_v[...] = jnp.zeros(y_v.shape, f32)

        def block(B, carry):
            fast = jnp.logical_and(B < NB, flag_s[B % 2] == 1)
            sup = jnp.logical_and(fast, B >= 2)

            @pl.when(B >= 2)
            def _():
                o_wait(B - 2)

            @pl.when(B == 2)
            def _():
                for w, g in [(2, 1), (0, 2), (1, 2), (2, 2), (0, 3), (1, 3), (2, 3)]:
                    f_copy(w, g).wait()

            with jax.named_scope("S_super"):
                @pl.when(sup)
                def _():
                    if only_super < 2:
                        superbody(B)

            @pl.when(jnp.logical_not(sup))
            def _():
                if only_super:
                    return

                def inner(g, c2):
                    step(4 * B + g, fast)
                    return c2

                lax.fori_loop(0, 4, inner, 0)

            @pl.when(B >= 2)
            def _():
                o_copy(B - 2, B % 2).start()

            return carry

        with jax.named_scope("S_main"):
            lax.fori_loop(0, NB + 2, block, 0)
        o_copy(NB - 2, 0).wait()
        o_copy(NB - 1, 1).wait()

    def call(A_x, A_wq, A_wk, A_wv, A_wo, B_x, B_w_gate, B_w_up, B_w_down, c, w_mod):
        xt = A_x.reshape(S, D).T
        hb = pl.BlockSpec(memory_space=pl.ANY)
        out = pl.pallas_call(
            kern,
            in_specs=[hb] * 10,
            out_specs=hb,
            out_shape=jax.ShapeDtypeStruct((D, S), bf16),
            scratch_shapes=[
                pltpu.VMEM((NB, D, TB), bf16),
                pltpu.VMEM((D, 6 * D), bf16),
                pltpu.VMEM((D, D), bf16),
                pltpu.VMEM((D, D), bf16),
                pltpu.VMEM((D, D), bf16),
                pltpu.VMEM((D, D), bf16),
                pltpu.VMEM((64, D), bf16),
                pltpu.VMEM((6, D, 128), f32),
                pltpu.VMEM((8, 128, 128), u32),
                pltpu.VMEM((8, 80, 256), f32),
                pltpu.VMEM((S // 2, 32), u32),
                pltpu.VMEM((KBE[-1], DH * 128), f32),
                pltpu.VMEM((4, 16, S), u32),
                pltpu.VMEM((8, NCP, 128, 256), bf16),
                pltpu.VMEM((4, 160, TB), f32),
                pltpu.VMEM((64, 640), u32),
                pltpu.VMEM((2, 64, 640), u32),
                pltpu.VMEM((2, D, TB), bf16),
                pltpu.VMEM((NB, 16, 256), f32),
                pltpu.VMEM((TB, 1280), bf16),
                pltpu.VMEM((2, 2 * NFT, TB, 128), f32),
                pltpu.VMEM((D, TB), f32),
                pltpu.VMEM((2, D, TB), f32),
                pltpu.VMEM((2, D, TB), bf16),
                pltpu.VMEM((4, D, FG), bf16),
                pltpu.VMEM((4, D, FG), bf16),
                pltpu.VMEM((4, D, FG), bf16),
                pltpu.VMEM((32, 128), f32),
                pltpu.VMEM((1, D), bf16),
                pltpu.VMEM((DH, D), bf16),
                pltpu.VMEM((DH, D), bf16),
                pltpu.SemaphoreType.DMA((NB,)),
                pltpu.SemaphoreType.DMA((10,)),
                pltpu.SemaphoreType.DMA((12,)),
                pltpu.SemaphoreType.DMA((2,)),
                pltpu.SMEM((2,), i32),
            ],
            compiler_params=pltpu.CompilerParams(vmem_limit_bytes=110 * 1024 * 1024),
            name="v18k",
        )(c, A_wk.T, A_wv.T, xt, A_wq, A_wo, B_w_gate, B_w_up, B_w_down.T, w_mod)
        return out.T.reshape(1, S, D)

    return call


_call = make()


@jax.jit
def pallas_adaLN_cond__grouped_kv_mqa__swiglu_ffn__prompt_kernel(A_x, A_wq, A_wk, A_wv, A_wo, B_x, B_w_gate, B_w_up, B_w_down, c, w_mod):
    return _call(A_x, A_wq, A_wk, A_wv, A_wo, B_x, B_w_gate, B_w_up, B_w_down, c, w_mod)
```

```python
import functools

import jax
import jax.numpy as jnp
from jax import lax
import jax.experimental.pallas as pl
import jax.experimental.pallas.tpu as pltpu

S, D, H, DH, F = 2048, 576, 32, 18, 4608
TB = 128
NB = S // TB
NCP = S // 256
FG = F // 4
NFT = FG // 128
EPS = 1e-5
LOG2E = 1.4426950408889634
QSCALE = DH ** -0.5 * LOG2E
TBOUND = 60.0
f32, bf16, u32, i32 = jnp.float32, jnp.bfloat16, jnp.uint32, jnp.int32
KT = [(0, 128), (128, 128), (256, 128), (384, 128), (512, 64)]
VSLOTS = [0, 4, 8, 12, 1, 5, 9, 3, 7, 11]
NVM = len(VSLOTS)
KORDER = ([(sl, hf) for sl in range(16) for hf in range(2) if not (hf == 1 and sl in VSLOTS)]
          + [(sl, 1) for sl in VSLOTS])
DR5 = [(0, 128), (128, 256), (256, 384), (384, 512), (512, 576)]
DR2 = [(0, 288), (288, 576)]
NT = (((1,), (1,)), ((), ()))
ATASKS = [(u, c) for u in range(8) for c in range(NCP)]
FSTART = {0: [(0, 0), (1, 0)], 1: [(2, 0), (0, 1), (1, 1)], 2: [(2, 1), (0, 2), (1, 2)],
          3: [(2, 2), (0, 3), (1, 3), (2, 3)]}
FWAIT = {6: [(0, 0), (1, 0)], 7: [(2, 0), (0, 1), (1, 1)]}
FWAIT2 = [(2, 1), (0, 2), (1, 2), (2, 2), (0, 3), (1, 3), (2, 3)]


def _bf(x):
    return pltpu.bitcast(x, bf16)


def _u32(x):
    return pltpu.bitcast(x.astype(bf16), u32)


def _stats_part(x, piv):
    d = (x - piv).reshape(x.shape[0] // 8, 8, TB)
    return jnp.sum(d, axis=0), jnp.sum(d * d, axis=0)


def _stats_fin(parts, piv):
    s1 = sum(p[0] for p in parts[1:]) + parts[0][0]
    s2 = sum(p[1] for p in parts[1:]) + parts[0][1]
    m1 = jnp.sum(s1, axis=0, keepdims=True) * (1.0 / D)
    m2 = jnp.sum(s2, axis=0, keepdims=True) * (1.0 / D)
    var = jnp.maximum(m2 - m1 * m1, 0.0)
    return piv + m1, lax.rsqrt(var + EPS)


def _stats(x):
    piv = x[0:1]
    return _stats_fin([_stats_part(x[r:r + 144], piv) for r in range(0, D, 144)], piv)


def _eye(n):
    return (lax.broadcasted_iota(i32, (n, n), 0) == lax.broadcasted_iota(i32, (n, n), 1)).astype(bf16)


def _mm4(w_ref, rhs):
    return jnp.concatenate([jnp.dot(w_ref[r:r + 144, :], rhs, preferred_element_type=f32)
                            for r in range(0, D, 144)], axis=0)


def _unorder(s):
    halves = []
    for hf in range(2):
        runs = []
        for sl in range(16):
            pos = KORDER.index((sl, hf))
            if runs and runs[-1][1] == pos:
                runs[-1][1] = pos + 1
            else:
                runs.append([pos, pos + 1])
        halves.append(jnp.concatenate([s[8 * a:8 * b] for a, b in runs], axis=0))
    return jnp.concatenate(halves, axis=1)


def _kernel(c_hbm, wkt_hbm, wvt_hbm, xt_hbm, wq_hbm, wo_hbm, wg_hbm, wu_hbm, wdt_hbm, wmod_hbm,
            out_hbm,
            x_v, wmod_v, wq_v, wo_v, wqt_v, wot_v, wkv_v, modc_v, q_v, qf_v, k_v, kb_v, vt_v,
            p_v, ot_v, h2_v, h2n_v, h2t_v, ln_v, ln2_v, a_v, acc_v, y_v, x1_v, o_v, wg_v, wu_v, wd_v, stat_v,
            c_ref, wkt_ref, wvt_ref,
            sem_x, sem_w, sem_f, sem_o, flag_s):
    def x_copy(b):
        return pltpu.make_async_copy(xt_hbm.at[:, pl.ds(b * TB, TB)], x_v.at[b], sem_x.at[b])

    cp_mod1 = pltpu.make_async_copy(wmod_hbm.at[:, pl.ds(0, 2 * D)], wmod_v.at[:, pl.ds(0, 2 * D)], sem_w.at[6])

    def wq_copy(j):
        return pltpu.make_async_copy(wq_hbm.at[pl.ds(j * 144, 144), :], wq_v.at[pl.ds(j * 144, 144), :],
                                     sem_w.at[2 + j])

    cp_mod2 = pltpu.make_async_copy(wmod_hbm.at[:, pl.ds(2 * D, 4 * D)], wmod_v.at[:, pl.ds(2 * D, 4 * D)],
                                    sem_w.at[0])
    cp_wo = pltpu.make_async_copy(wo_hbm, wo_v, sem_w.at[1])

    def f_copy(w, g):
        src, dst = ((wg_hbm, wg_v), (wu_hbm, wu_v), (wdt_hbm, wd_v))[w]
        return pltpu.make_async_copy(src.at[:, pl.ds(g * FG, FG)], dst.at[g], sem_f.at[w * 4 + g])

    def o_copy(b, slot):
        return pltpu.make_async_copy(o_v.at[slot], out_hbm.at[:, pl.ds(pl.multiple_of(b * TB, TB), TB)],
                                     sem_o.at[slot])

    small = [pltpu.make_async_copy(src, dst, sem_w.at[7 + i]) for i, (src, dst) in enumerate(
        [(c_hbm, c_ref), (wkt_hbm, wkt_ref), (wvt_hbm, wvt_ref)])]
    for cp in small:
        cp.start()
    for b in range(4):
        x_copy(b).start()
    cp_mod1.start()
    for cp in small:
        cp.wait()

    c = c_ref[...].astype(f32)
    sc = jnp.broadcast_to((c * jax.nn.sigmoid(c)).astype(bf16), (16, D))
    wkv_v[...] = jnp.zeros(wkv_v.shape, bf16)
    wkv_v[0:DH, :] = wkt_ref[...]
    wkv_v[32:32 + DH, :] = wvt_ref[...]

    def mod_cols(c0, n):
        m = jnp.dot(sc, wmod_v[:, c0:c0 + n], preferred_element_type=f32)[0:1]
        return jnp.broadcast_to(m, (128, n)).T

    def ln1_stats(b):
        m, r = _stats(x_v[b].astype(f32))
        ln_v[b, 0:1, 0:128] = m
        ln_v[b, 1:2, 0:128] = r

    for b in range(4):
        x_copy(b).wait()
    for b in range(4, 8):
        x_copy(b).start()
    for b in range(4):
        ln1_stats(b)
    cp_mod1.wait()
    for b in range(8, NB):
        x_copy(b).start()
    for j in range(4):
        wq_copy(j).start()
    m1 = mod_cols(0, 2 * D)
    modc_v[0] = m1[0:D]
    modc_v[1] = 1.0 + m1[D:2 * D]

    def h1_of(b):
        xn = (x_v[b].astype(f32) - ln_v[b, 0:1, 0:128]) * ln_v[b, 1:2, 0:128]
        return (xn * modc_v[1] + modc_v[0]).astype(bf16)

    def kv_s1(b):
        if b >= 4:
            ln1_stats(b)
        return jnp.dot(wkv_v[...], h1_of(b), preferred_element_type=f32)

    def kv_s2(b, kvt, kn, va):
        row32 = lax.broadcasted_iota(i32, (32, TB), 0)
        ktb = kvt[0:32].astype(bf16)
        kt = ktb.astype(f32)
        kn = jnp.maximum(kn, jnp.sum(kt * kt, axis=0, keepdims=True))
        va = jnp.maximum(va, jnp.abs(kvt[32:64]))
        for v in range(4):
            vt = kvt[32 - 2 * v:64 - 2 * v]
            vt = jnp.where(row32 == (0 if v == 3 else 23), 1.0, vt)
            vt_v[v, :, b * TB:(b + 1) * TB] = _u32(vt)
        return lax.dot_general(_eye(128), ktb, NT, preferred_element_type=f32), kn, va

    def kv_s3(cp, pair):
        k_v[cp * 128:(cp + 1) * 128, :] = _u32(
            jnp.concatenate([pair[hf][8 * sl:8 * sl + 8] for sl, hf in KORDER], axis=0))

    def kv_s4(cp, half):
        c0, c1 = half * 9 * 128, (half + 1) * 9 * 128
        esel = (lax.broadcasted_iota(i32, (32, 9 * 128), 0)
                == lax.shift_right_logical(lax.broadcasted_iota(i32, (32, 9 * 128), 1), 7) + 9 * half).astype(bf16)
        kv = _bf(k_v[(cp + 1) * 128 - 4 * NVM:(cp + 1) * 128, :])
        kb_v[cp * 8 * NVM:(cp + 1) * 8 * NVM, c0:c1] = jnp.dot(kv, esel, preferred_element_type=f32)

    def q_block(h1, slot):
        qt = _mm4(wqt_v, h1) * QSCALE
        qr = qt.astype(bf16).astype(f32)
        z8 = jnp.zeros((8, TB), f32)
        qz = jnp.concatenate([qr, z8], axis=0)
        row8 = lax.broadcasted_iota(i32, (8, TB), 0)
        qn = None
        for g in range(4):
            r0 = 144 * g
            wins = []
            for u in range(8):
                w = qz[r0 + DH * u:r0 + DH * u + 24]
                wins += [w, z8]
                sq = w * w
                t = sq[0:8] + sq[8:16] + jnp.where(row8 < DH - 16, sq[16:24], 0.0)
                t = jnp.sum(t, axis=0, keepdims=True)
                qn = t if qn is None else jnp.maximum(qn, t)
            q_v[slot * 4 + g] = _u32(jnp.concatenate(wins, axis=0))
            qf_v[slot * 4 + g, 0:72, 0:128] = qr[r0:r0 + 72]
            qf_v[slot * 4 + g, 0:72, 128:256] = qr[r0 + 72:r0 + 144]
        return qn

    def set_flag(qn, slot):
        ok = jnp.where(qn * stat_v[0:1, :] <= stat_v[1:2, :], 1.0, 0.0)
        flag_s[slot] = (jnp.min(ok) > 0.5).astype(i32)

    kn = jnp.zeros((1, TB), f32)
    va = jnp.zeros((32, TB), f32)
    kvts, ktoks = {}, {}
    for i in range(NB + 5):
        if i in (4, 8, 12):
            for b in range(i, i + 4):
                x_copy(b).wait()
        if i == 12:
            for j in range(4):
                wq_copy(j).wait()
            cp_mod2.start()
            cp_wo.start()
            wqt_v[...] = wq_v[...].T
        if i < NB:
            kvts[i] = kv_s1(i)
        if 0 <= i - 1 < NB:
            ktoks[i - 1], kn, va = kv_s2(i - 1, kvts.pop(i - 1), kn, va)
        if i == NB:
            qn0 = q_block(h1_of(0), 0)
        if i >= 3 and i % 2 == 1 and (i - 3) // 2 < NCP:
            cp = (i - 3) // 2
            kv_s3(cp, [ktoks.pop(2 * cp), ktoks.pop(2 * cp + 1)])
        if i >= 3 and (i - 3) // 2 < NCP:
            kv_s4((i - 3) // 2, (i - 3) % 2)
    kn2 = jnp.max(kn, axis=1, keepdims=True)
    vrow = jnp.max(va, axis=1, keepdims=True)
    v_ok = jnp.logical_or(vrow == 0.0, jnp.logical_and(vrow >= 2.0 ** -40, vrow <= 2.0 ** 40))
    v_bad = jnp.max(jnp.where(v_ok, 0.0, 1.0), axis=0, keepdims=True)
    lim = jnp.where(v_bad > 0.0, -1.0, TBOUND * TBOUND / 1.02)
    stat_v[0:1, :] = jnp.broadcast_to(kn2, (1, 128))
    stat_v[1:2, :] = jnp.broadcast_to(lim, (1, 128))
    set_flag(qn0, 0)

    def late_setup():
        cp_mod2.wait()
        cp_wo.wait()
        wot_v[...] = wo_v[...].T
        for i in range(2):
            m2 = mod_cols((2 + 2 * i) * D, 2 * D)
            modc_v[2 + 2 * i] = m2[0:D] + float(i)
            modc_v[3 + 2 * i] = m2[D:2 * D]
        set_flag(q_block(h1_of(1), 1), 1)

    class Unit:
        def __init__(self, qi, gb, gc, gd, par, y_first=False, drs=DR5):
            self.qi, self.gb, self.gc, self.gd, self.par = qi, gb, gc, gd, par
            self.y_first, self.drs = y_first, drs
            self.o = [None] * 8
            self.carry = None
            self.qrows = {}

        def score_a(self, u, c):
            return jnp.dot(_bf(k_v[c * 128:c * 128 + 64, :]), _bf(q_v[self.qi, 16 * u:16 * u + 16, :]),
                           preferred_element_type=f32)

        def score_b(self, u, c, nv):
            return jnp.dot(_bf(k_v[c * 128 + 64:(c + 1) * 128 - 4 * nv, :]),
                           _bf(q_v[self.qi, 16 * u:16 * u + 16, :]), preferred_element_type=f32)

        def score_end(self, u, c, nv, sa, sb):
            if u not in self.qrows:
                lo = (u // 4) * 128
                q0 = DH * (u % 4)
                self.qrows[u] = jnp.concatenate(
                    [jnp.broadcast_to(qf_v[self.qi, q0 + d:q0 + d + 1, lo:lo + 128], (8, TB)) for d in range(DH)],
                    axis=1)[None]
            r1 = (c + 1) * 8 * NVM
            prod = kb_v[r1 - 8 * nv:r1, :].reshape(nv, 8, DH * 128) * self.qrows[u]
            sv = prod[:, :, 0:256]
            for d in range(1, DH // 2):
                sv = sv + prod[:, :, d * 256:(d + 1) * 256]
            sv = sv[:, :, 0:128] + sv[:, :, 128:256]
            s = jnp.concatenate([sa, sb, sv.reshape(8 * nv, TB)], axis=0)
            p_v[u, c] = jnp.exp2(_unorder(s)).astype(bf16)

        def pv(self, u, c, hf):
            o = self.o
            k0 = c * 256 + hf * 128
            oc = jnp.dot(_bf(vt_v[u % 4, :, k0:k0 + 128]), p_v[u, c, :, hf * 128:(hf + 1) * 128],
                         preferred_element_type=f32)[0:24]
            o[u] = oc if o[u] is None else o[u] + oc
            if c == NCP - 1 and hf == 1:
                row24 = lax.broadcasted_iota(i32, (24, TB), 0)
                r1 = 0 if u % 4 == 3 else 23
                on = jnp.where(row24 == r1, 0.0, o[u] * (1.0 / o[u][r1:r1 + 1]))
                base = 16 * u + 8 * (u // 4)
                first = on[0:8] if u % 4 == 0 else on[0:8] + self.carry
                ot_v[self.gb, base:base + 8, :] = first
                if u % 4 == 3:
                    ot_v[self.gb, base + 8:base + 24, :] = on[8:24]
                else:
                    ot_v[self.gb, base + 8:base + 16, :] = on[8:16]
                    self.carry = on[16:24]

        def piece(self, kind, f, j):
            cols = slice(f * 128, (f + 1) * 128)
            par = self.par
            if kind in "gu":
                w_ref = wg_v if kind == "g" else wu_v
                ai = 2 * f + (kind == "u")
                k0, kn_ = KT[j]
                r = jnp.dot(_bf(h2_v[:, k0:k0 + kn_]), w_ref[self.gc, k0:k0 + kn_, cols],
                            preferred_element_type=f32)
                if j > 0:
                    r = r + acc_v[par, ai]
                if j < 4:
                    acc_v[par, ai] = r
                elif kind == "g":
                    acc_v[par, ai] = r * pl.reciprocal(1.0 + jnp.exp2(r * (-LOG2E)), approx=True)
                else:
                    a_v[:, cols] = (acc_v[par, ai - 1] * r).astype(bf16)
            else:
                ra, rb = self.drs[j]
                yc = lax.dot_general(wd_v[self.gd, ra:rb, cols], a_v[:, cols], NT, preferred_element_type=f32)
                if self.y_first and f == 0:
                    y_v[ra:rb, :] = yc
                else:
                    y_v[ra:rb, :] += yc

        def ffn_list(self, C, Dn):
            gl = []
            if C:
                gl = [(k, f, j) for j in range(4) for f in range(NFT) for k in "gu"]
                for i in range(NFT + 1):
                    gl += ([("g", i, 4)] if i < NFT else []) + ([("u", i - 1, 4)] if i >= 1 else [])
            dl = []
            nd = len(self.drs)
            if Dn:
                dl = [("d", f, j) for f in range(NFT)
                      for j in (range(nd) if f % 2 == 0 else range(nd - 1, -1, -1))]
            fp = []
            di = 0
            for m, gp in enumerate(gl):
                assert gp[2] < 4 or di == len(dl)
                fp.append(gp)
                while di < len(dl) and (di * 72 <= m * len(dl)
                                        or (di > 0 and dl[di][2] == 4 and dl[di - 1][2] == 4)):
                    fp.append(dl[di])
                    di += 1
            fp += dl[di:]
            return [(self.drs[p[2]][1] - self.drs[p[2]][0] if p[0] == "d" else 128,
                     functools.partial(self.piece, *p), p) for p in fp]

    def body(n, A, B, C, Dn):
        un = Unit(n % 8, (n + 3) % 4, (n + 2) % 4, (n + 1) % 4, n % 2)
        for u, c in (ATASKS if (A or B) else []):
            if B:
                un.pv(u, c, 0)
                un.pv(u, c, 1)
            if A:
                nv = 4 + 2 * (c % 2)
                un.score_end(u, c, nv, un.score_a(u, c), un.score_b(u, c, nv))
        for _, thunk, _ in un.ffn_list(C, Dn):
            thunk()

    def e1_wo(b):
        ot = jnp.concatenate([ot_v[g, 0:144, :] for g in range(4)], axis=0).astype(bf16)
        att = _mm4(wot_v, ot)
        x1 = x_v[b].astype(f32) + modc_v[2] * att
        x1_v[b % 2] = x1
        return _stats(x1)

    def e1_wo_piece(b, r, j, st):
        k0, kn_ = KT[j]
        segs = []
        for g in range(4):
            lo, hi = max(k0, 144 * g), min(k0 + kn_, 144 * g + 144)
            if lo < hi:
                segs.append(ot_v[g, lo - 144 * g:hi - 144 * g, :])
        ot = jnp.concatenate(segs, axis=0).astype(bf16)
        rows = slice(144 * r, 144 * r + 144)
        res = jnp.dot(wot_v[rows, k0:k0 + kn_], ot, preferred_element_type=f32)
        if j > 0:
            res = res + x1_v[b % 2, rows, :]
        if j == 4:
            res = x_v[b, rows, :].astype(f32) + modc_v[2, rows, :] * res
            if r == 0:
                st["piv"] = res[0:1]
            st.setdefault("parts", []).append(_stats_part(res, st["piv"]))
        x1_v[b % 2, rows, :] = res

    def e1_q(b, m, r):
        ln2_v[b % 2, 0:1, 0:128] = m
        ln2_v[b % 2, 1:2, 0:128] = r
        qn = q_block(h1_of(jnp.minimum(b + 2, NB - 1)), b % 2)
        for q0 in range(0, D, 144):
            rows = slice(q0, q0 + 144)
            xn = (x1_v[b % 2, rows, :] - ln2_v[b % 2, 0:1, 0:128]) * ln2_v[b % 2, 1:2, 0:128]
            h2t_v[b % 2, rows, :] = (xn * modc_v[4, rows, :] + modc_v[3, rows, :]).astype(bf16)
        return qn

    def e1_tr(b, j):
        k0, kn_ = KT[j]
        h2 = lax.dot_general(_eye(128), h2t_v[b % 2, k0:k0 + kn_, :], NT, preferred_element_type=f32)
        h2n_v[b % 2, :, k0:k0 + kn_] = _u32(h2)

    def h2_switch(b, j):
        k0, kn_ = KT[j]
        h2_v[:, k0:k0 + kn_] = h2n_v[b % 2, :, k0:k0 + kn_]

    def e2_core(b):
        o_v[b % 2] = (x1_v[b % 2] + modc_v[5] * y_v[...]).astype(bf16)

    def superbody(B):
        qb = (B % 2) * 4
        units = [Unit(qb + g, (g + 3) % 4, (g + 2) % 4, (g + 1) % 4, B % 2, y_first=(g == 3), drs=DR2)
                 for g in range(4)]
        l1 = units[1].ffn_list(1, 1)
        for j in range(5):
            i = max(k for k, e in enumerate(l1) if e[2][0] in "gu" and e[2][2] == j)
            l1.insert(i + 1, (0, functools.partial(h2_switch, B - 1, j), ("s", 0, j)))
        l2 = units[2].ffn_list(1, 1)
        last_d = max(i for i, e in enumerate(l2) if e[2][0] == "d")
        l2.insert(last_d + 1, (0, functools.partial(e2_core, B - 2), ("e", 0, 0)))
        fl = units[0].ffn_list(1, 1) + l1 + l2 + units[3].ffn_list(1, 1)
        hist = []
        tasks = [(un, u, c) for un in units for u, c in ATASKS]
        nt = len(tasks)
        col1 = []
        for t in range(nt + 1):
            if t > 0:
                col1.append(("b", t - 1))
            if t < nt:
                col1 += [("p", t, 0), ("p", t, 1)]
        sa, sb, nvs = {}, {}, {}
        pdone = [False] * nt
        fin = [0]

        def finish():
            while fin[0] < nt and fin[0] in sa and fin[0] in sb and pdone[fin[0]]:
                un, u, c = tasks[fin[0]]
                un.score_end(u, c, nvs[fin[0]], sa.pop(fin[0]), sb.pop(fin[0]))
                fin[0] += 1

        def take_f():
            rows, thunk, p = fl.pop(0)
            hist.append(p)
            thunk()
            while fl and fl[0][0] == 0:
                _, thunk, p = fl.pop(0)
                assert p[0] != "s" or ("t", 0, p[2]) in hist
                thunk()
            return rows

        def first_free():
            return min((0, 2, 3, 1), key=lambda m: T[m])

        T = [64, 0, 64, 64]
        i0 = 0
        qn = None
        wo_at = 64 + 3
        e1_at = 10 ** 6
        wst = {}
        xbef = xleft = 1
        while i0 < nt or col1 or fl:
            k = first_free()
            if i0 == wo_at and not wst:
                assert pdone[63]
                wst["on"] = True
                for i, (j, r) in enumerate((j, r) for j in range(5) for r in range(4)):
                    fl.insert(i, (144, functools.partial(e1_wo_piece, B - 1, r, j, wst), ("w", r, j)))
            if e1_at > nt and len(wst.get("parts", ())) == 4:
                e1_at = i0
            if qn is None and i0 == e1_at and k == 0 and xbef:
                T[0] += take_f()
                xbef -= 1
                continue
            if qn is None and i0 == e1_at and k == 0:
                qn = e1_q(B - 1, *_stats_fin(wst["parts"], wst["piv"]))
                for j in range(5):
                    fl.insert(j, (128, functools.partial(e1_tr, B - 1, j), ("t", 0, j)))
                set_flag(qn, (B - 1) % 2)
                for _ in range(20):
                    T[first_free()] += 144
                continue
            if k == 0 and qn is not None and xleft and fl:
                T[0] += take_f()
                xleft -= 1
            elif k == 0 and i0 < nt:
                un, u, c = tasks[i0]
                sa[i0] = un.score_a(u, c)
                i0 += 1
                T[0] += 128
            elif k == 1 and col1:
                it = col1[0]
                due = T[0] + 128 * (it[1] - i0) - (64 if it[0] == "p" and it[2] == 0 else 0)
                lead = due - T[1]
                blocked = qn is None and it[1] > e1_at
                if fl and (blocked or (it[0] != "p" or it[2] == 0) and lead - 192 >= fl[0][0]):
                    T[1] += take_f()
                else:
                    col1.pop(0)
                    un, u, c = tasks[it[1]]
                    if it[0] == "p":
                        if it[1] >= 64 and c == NCP - 1:
                            lim = 144 * ((it[1] - 64) // 64) + DH * (u + 1) + 8
                            assert wst and not any(e[2][0] == "w" and KT[e[2][2]][0] < lim for e in fl)
                        un.pv(u, c, it[2])
                        pdone[it[1]] = it[2] == 1
                        T[1] += 32
                    else:
                        near = hist[-2:] + [e[2] for e in fl[:2]]
                        nv = NVM
                        if any(p[0] == "g" and p[2] == 4 for p in near):
                            nv = min(nv, 8)
                        if any(p[0] == "w" for p in near):
                            nv = min(nv, 6 if any(p[0] == "w" and p[2] == 4 for p in near) else 8)
                        if e1_at <= it[1] < e1_at + 4:
                            nv = min(nv, 6)
                        if it[1] >= nt - 2:
                            nv = min(nv, 4)
                        nvs[it[1]] = nv
                        sb[it[1]] = un.score_b(u, c, nv)
                        T[1] += 128 - 8 * nv
            elif fl:
                T[k] += take_f()
            else:
                T[k] = 10 ** 9
            finish()
        assert fin[0] == nt

    def a_slow(n):
        qi = n % 8

        def head(u, carry):
            w = pl.multiple_of(16 * u, 16)
            s = jnp.dot(_bf(k_v[...]), _bf(q_v[qi, pl.ds(w, 16), :]), preferred_element_type=f32)
            p = jnp.exp2(s - jnp.max(s, axis=0, keepdims=True))
            for c in range(NCP):
                p_v[u, c] = _unorder(p[c * 256:(c + 1) * 256]).astype(bf16)
            return carry

        lax.fori_loop(0, 8, head, 0)

    def step(n, fast):
        @pl.when(n <= 8)
        def _():
            for m, starts in FSTART.items():
                @pl.when(n == m)
                def _():
                    for w, g in starts:
                        f_copy(w, g).start()

            @pl.when(n == 3)
            def _():
                late_setup()

            for m, waits in FWAIT.items():
                @pl.when(n == m)
                def _():
                    for w, g in waits:
                        f_copy(w, g).wait()

        @pl.when(fast)
        def _():
            body(n, 1, 1, 0, 0)

        @pl.when(jnp.logical_not(fast))
        def _():
            @pl.when(jnp.logical_and(n >= 1, n <= 64))
            def _():
                body(n, 0, 1, 0, 0)

            @pl.when(n < 64)
            def _():
                a_slow(n)

        @pl.when(jnp.logical_and(n >= 7, n <= 69))
        def _():
            body(n, 0, 0, 1, 1)

        @pl.when(n == 70)
        def _():
            body(n, 0, 0, 0, 1)

        @pl.when(n == 6)
        def _():
            body(n, 0, 0, 1, 0)
            y_v[...] = jnp.zeros(y_v.shape, f32)

        @pl.when(jnp.logical_and(n % 4 == 0, jnp.logical_and(n >= 4, n <= 64)))
        def _():
            b = n // 4 - 1
            set_flag(e1_q(b, *e1_wo(b)), b % 2)
            for j in range(5):
                e1_tr(b, j)

        @pl.when(jnp.logical_and(n % 4 == 1, jnp.logical_and(n >= 5, n <= 65)))
        def _():
            for j in range(5):
                h2_switch(n // 4 - 1, j)

        @pl.when(jnp.logical_and(n % 4 == 2, n >= 10))
        def _():
            e2_core(n // 4 - 2)
            y_v[...] = jnp.zeros(y_v.shape, f32)

    def block(B, carry):
        fast = jnp.logical_and(B < NB, flag_s[B % 2] == 1)
        sup = jnp.logical_and(fast, B >= 2)

        @pl.when(B >= 4)
        def _():
            o_copy(B - 4, B % 2).wait()

        @pl.when(B == 2)
        def _():
            for w, g in FWAIT2:
                f_copy(w, g).wait()

        @pl.when(sup)
        def _():
            superbody(B)

        @pl.when(jnp.logical_not(sup))
        def _():
            def inner(g, c2):
                step(4 * B + g, fast)
                return c2

            lax.fori_loop(0, 4, inner, 0)

        @pl.when(B >= 2)
        def _():
            o_copy(B - 2, B % 2).start()

        return carry

    lax.fori_loop(0, NB + 2, block, 0)
    o_copy(NB - 2, 0).wait()
    o_copy(NB - 1, 1).wait()


@jax.jit
def pallas_adaLN_cond__grouped_kv_mqa__swiglu_ffn__prompt_kernel(
        A_x, A_wq, A_wk, A_wv, A_wo, B_x, B_w_gate, B_w_up, B_w_down, c, w_mod):
    hb = pl.BlockSpec(memory_space=pl.ANY)
    out = pl.pallas_call(
        _kernel,
        in_specs=[hb] * 10,
        out_specs=hb,
        out_shape=jax.ShapeDtypeStruct((D, S), bf16),
        scratch_shapes=[
            pltpu.VMEM((NB, D, TB), bf16),
            pltpu.VMEM((D, 6 * D), bf16),
            pltpu.VMEM((D, D), bf16),
            pltpu.VMEM((D, D), bf16),
            pltpu.VMEM((D, D), bf16),
            pltpu.VMEM((D, D), bf16),
            pltpu.VMEM((64, D), bf16),
            pltpu.VMEM((6, D, 128), f32),
            pltpu.VMEM((8, 128, 128), u32),
            pltpu.VMEM((8, 80, 256), f32),
            pltpu.VMEM((S // 2, 32), u32),
            pltpu.VMEM((NCP * 8 * NVM, DH * 128), f32),
            pltpu.VMEM((4, 16, S), u32),
            pltpu.VMEM((8, NCP, 128, 256), bf16),
            pltpu.VMEM((4, 160, TB), f32),
            pltpu.VMEM((64, 640), u32),
            pltpu.VMEM((2, 64, 640), u32),
            pltpu.VMEM((2, D, TB), bf16),
            pltpu.VMEM((NB, 16, 256), f32),
            pltpu.VMEM((2, 16, 256), f32),
            pltpu.VMEM((TB, 1280), bf16),
            pltpu.VMEM((2, 2 * NFT, TB, 128), f32),
            pltpu.VMEM((D, TB), f32),
            pltpu.VMEM((2, D, TB), f32),
            pltpu.VMEM((2, D, TB), bf16),
            pltpu.VMEM((4, D, FG), bf16),
            pltpu.VMEM((4, D, FG), bf16),
            pltpu.VMEM((4, D, FG), bf16),
            pltpu.VMEM((32, 128), f32),
            pltpu.VMEM((1, D), bf16),
            pltpu.VMEM((DH, D), bf16),
            pltpu.VMEM((DH, D), bf16),
            pltpu.SemaphoreType.DMA((NB,)),
            pltpu.SemaphoreType.DMA((10,)),
            pltpu.SemaphoreType.DMA((12,)),
            pltpu.SemaphoreType.DMA((2,)),
            pltpu.SMEM((2,), i32),
        ],
        compiler_params=pltpu.CompilerParams(vmem_limit_bytes=110 * 1024 * 1024),
    )(c, A_wk.T, A_wv.T, A_x.reshape(S, D).T, A_wq, A_wo, B_w_gate, B_w_up, B_w_down.T, w_mod)
    return out.T.reshape(1, S, D)
```

```python
import functools

import jax
import jax.numpy as jnp
from jax import lax
import jax.experimental.pallas as pl
import jax.experimental.pallas.tpu as pltpu

S, D, H, DH, F = 2048, 576, 32, 18, 4608
TB = 128
NB = S // TB
FG = F // 4
NFT = FG // 128
EPS = 1e-5
LOG2E = 1.4426950408889634
QSCALE = DH ** -0.5 * LOG2E
TBOUND = 60.0
f32, bf16, u32, i32 = jnp.float32, jnp.bfloat16, jnp.uint32, jnp.int32
KT = [(0, 128), (128, 128), (256, 128), (384, 128), (512, 64)]
KV = 640
DR5 = [(0, 128), (128, 256), (256, 384), (384, 512), (512, 576)]
DR2 = [(0, 288), (288, 576)]
NT = (((1,), (1,)), ((), ()))
FSTART = {0: [(0, 0), (1, 0)], 1: [(2, 0), (0, 1), (1, 1)], 2: [(2, 1), (0, 2), (1, 2)],
          3: [(2, 2), (0, 3), (1, 3), (2, 3)]}
FWAIT = {6: [(0, 0), (1, 0)], 7: [(2, 0), (0, 1), (1, 1)]}
FWAIT2 = [(2, 1), (0, 2), (1, 2), (2, 2), (0, 3), (1, 3), (2, 3)]


def _bf(x):
    return pltpu.bitcast(x, bf16)


def _u32(x):
    return pltpu.bitcast(x.astype(bf16), u32)


def _stats_part(x, piv):
    d = (x - piv).reshape(x.shape[0] // 8, 8, TB)
    return jnp.sum(d, axis=0), jnp.sum(d * d, axis=0)


def _stats_fin(parts, piv):
    s1 = sum(p[0] for p in parts[1:]) + parts[0][0]
    s2 = sum(p[1] for p in parts[1:]) + parts[0][1]
    m1 = jnp.sum(s1, axis=0, keepdims=True) * (1.0 / D)
    m2 = jnp.sum(s2, axis=0, keepdims=True) * (1.0 / D)
    var = jnp.maximum(m2 - m1 * m1, 0.0)
    return piv + m1, lax.rsqrt(var + EPS)


def _stats(x):
    piv = x[0:1]
    return _stats_fin([_stats_part(x[r:r + 144], piv) for r in range(0, D, 144)], piv)


def _eye(n):
    return (lax.broadcasted_iota(i32, (n, n), 0) == lax.broadcasted_iota(i32, (n, n), 1)).astype(bf16)


def _mm4(w_ref, rhs):
    return jnp.concatenate([jnp.dot(w_ref[r:r + 144, :], rhs, preferred_element_type=f32)
                            for r in range(0, D, 144)], axis=0)


def _kernel(c_hbm, wkt_hbm, wvt_hbm, xt_hbm, wq_hbm, wo_hbm, wg_hbm, wu_hbm, wdt_hbm, wmod_hbm,
            out_hbm,
            x_v, wmod_v, wq_v, wo_v, wqt_v, wot_v, wkv_v, modc_v, q_v, qf_v, k_v, kb_v, vt_v,
            p_v, ot_v, h2_v, h2n_v, h2t_v, ln_v, ln2_v, a_v, acc_v, y_v, x1_v, o_v, wg_v, wu_v, wd_v, stat_v,
            c_ref, wkt_ref, wvt_ref,
            sem_x, sem_w, sem_f, sem_o, flag_s):
    def x_copy(b):
        return pltpu.make_async_copy(xt_hbm.at[:, pl.ds(b * TB, TB)], x_v.at[b], sem_x.at[b])

    cp_mod1 = pltpu.make_async_copy(wmod_hbm.at[:, pl.ds(0, 2 * D)], wmod_v.at[:, pl.ds(0, 2 * D)], sem_w.at[6])

    def wq_copy(j):
        return pltpu.make_async_copy(wq_hbm.at[pl.ds(j * 144, 144), :], wq_v.at[pl.ds(j * 144, 144), :],
                                     sem_w.at[2 + j])

    cp_mod2 = pltpu.make_async_copy(wmod_hbm.at[:, pl.ds(2 * D, 4 * D)], wmod_v.at[:, pl.ds(2 * D, 4 * D)],
                                    sem_w.at[0])
    cp_wo = pltpu.make_async_copy(wo_hbm, wo_v, sem_w.at[1])

    def f_copy(w, g):
        src, dst = ((wg_hbm, wg_v), (wu_hbm, wu_v), (wdt_hbm, wd_v))[w]
        return pltpu.make_async_copy(src.at[:, pl.ds(g * FG, FG)], dst.at[g], sem_f.at[w * 4 + g])

    def o_copy(b, slot):
        return pltpu.make_async_copy(o_v.at[slot], out_hbm.at[:, pl.ds(pl.multiple_of(b * TB, TB), TB)],
                                     sem_o.at[slot])

    small = [pltpu.make_async_copy(src, dst, sem_w.at[7 + i]) for i, (src, dst) in enumerate(
        [(c_hbm, c_ref), (wkt_hbm, wkt_ref), (wvt_hbm, wvt_ref)])]
    for cp in small:
        cp.start()
    for b in range(4):
        x_copy(b).start()
    cp_mod1.start()
    for cp in small:
        cp.wait()

    c = c_ref[...].astype(f32)
    sc = jnp.broadcast_to((c * jax.nn.sigmoid(c)).astype(bf16), (16, D))
    wkv_v[...] = jnp.zeros(wkv_v.shape, bf16)
    wkv_v[0:DH, :] = wkt_ref[...]
    wkv_v[32:32 + DH, :] = wvt_ref[...]

    def mod_cols(c0, n):
        m = jnp.dot(sc, wmod_v[:, c0:c0 + n], preferred_element_type=f32)[0:1]
        return jnp.broadcast_to(m, (128, n)).T

    def ln1_stats(b):
        m, r = _stats(x_v[b].astype(f32))
        ln_v[b, 0:1, 0:128] = m
        ln_v[b, 1:2, 0:128] = r

    for b in range(4):
        x_copy(b).wait()
    for b in range(4, 8):
        x_copy(b).start()
    for b in range(4):
        ln1_stats(b)
    cp_mod1.wait()
    for b in range(8, NB):
        x_copy(b).start()
    for j in range(4):
        wq_copy(j).start()
    m1 = mod_cols(0, 2 * D)
    modc_v[0] = m1[0:D]
    modc_v[1] = 1.0 + m1[D:2 * D]

    def h1_of(b):
        xn = (x_v[b].astype(f32) - ln_v[b, 0:1, 0:128]) * ln_v[b, 1:2, 0:128]
        return (xn * modc_v[1] + modc_v[0]).astype(bf16)

    def kv_s1(b):
        if b >= 4:
            ln1_stats(b)
        return jnp.dot(wkv_v[...], h1_of(b), preferred_element_type=f32)

    def kv_s2(b, kvt, kn, va):
        row24 = lax.broadcasted_iota(i32, (24, TB), 0)
        ktb = kvt[0:32].astype(bf16)
        kt = ktb.astype(f32)
        kn = jnp.maximum(kn, jnp.sum(kt * kt, axis=0, keepdims=True))
        va = jnp.maximum(va, jnp.abs(kvt[32:64]))
        for v in range(4):
            vt = kvt[32 - 2 * v:56 - 2 * v]
            vt_v[v, :, b * TB:(b + 1) * TB] = jnp.where(row24 == (0 if v == 3 else 23), 1.0, vt)
        kt128 = jnp.concatenate([ktb, jnp.zeros((96, TB), bf16)], axis=0)
        k_v[b * 64:(b + 1) * 64, :] = _u32(lax.dot_general(_eye(128), kt128, NT, preferred_element_type=f32))
        return kn, va

    def kv_s4(b, part):
        c0, c1 = part * 6 * 128, (part + 1) * 6 * 128
        esel = (lax.broadcasted_iota(i32, (32, 6 * 128), 0)
                == lax.shift_right_logical(lax.broadcasted_iota(i32, (32, 6 * 128), 1), 7) + 6 * part).astype(bf16)
        kb_v[b * TB:(b + 1) * TB, c0:c1] = jnp.dot(_bf(k_v[b * 64:(b + 1) * 64, 0:32]), esel,
                                                   preferred_element_type=f32)

    def q_block(h1, slot):
        qt = _mm4(wqt_v, h1) * QSCALE
        qr = qt.astype(bf16).astype(f32)
        z8 = jnp.zeros((8, TB), f32)
        qz = jnp.concatenate([qr, z8], axis=0)
        row8 = lax.broadcasted_iota(i32, (8, TB), 0)
        qn = None
        for g in range(4):
            r0 = 144 * g
            wins = []
            for u in range(8):
                w = qz[r0 + DH * u:r0 + DH * u + 24]
                wins += [w, z8]
                sq = w * w
                t = sq[0:8] + sq[8:16] + jnp.where(row8 < DH - 16, sq[16:24], 0.0)
                t = jnp.sum(t, axis=0, keepdims=True)
                qn = t if qn is None else jnp.maximum(qn, t)
            q_v[slot * 4 + g] = _u32(jnp.concatenate(wins, axis=0))
            qf_v[slot * 4 + g, 0:72, 0:128] = qr[r0:r0 + 72]
            qf_v[slot * 4 + g, 0:72, 128:256] = qr[r0 + 72:r0 + 144]
        return qn

    def set_flag(qn, slot):
        ok = jnp.where(qn * stat_v[0:1, :] <= stat_v[1:2, :], 1.0, 0.0)
        flag_s[slot] = (jnp.min(ok) > 0.5).astype(i32)

    kn = jnp.zeros((1, TB), f32)
    va = jnp.zeros((32, TB), f32)
    kvts = {}
    kbq = [(b, part) for b in range(KV // TB) for part in range(3)]
    for i in range(NB + 5):
        if i in (4, 8, 12):
            for b in range(i, i + 4):
                x_copy(b).wait()
        if i == 12:
            for j in range(4):
                wq_copy(j).wait()
            cp_mod2.start()
            cp_wo.start()
            wqt_v[...] = wq_v[...].T
        if i < NB:
            kvts[i] = kv_s1(i)
        if 0 <= i - 1 < NB:
            kn, va = kv_s2(i - 1, kvts.pop(i - 1), kn, va)
        if i == NB:
            qn0 = q_block(h1_of(0), 0)
        if kbq and kbq[0][0] + 2 <= i:
            kv_s4(*kbq.pop(0))
    assert not kbq
    kn2 = jnp.max(kn, axis=1, keepdims=True)
    vrow = jnp.max(va, axis=1, keepdims=True)
    v_ok = jnp.logical_or(vrow == 0.0, jnp.logical_and(vrow >= 2.0 ** -40, vrow <= 2.0 ** 40))
    v_bad = jnp.max(jnp.where(v_ok, 0.0, 1.0), axis=0, keepdims=True)
    lim = jnp.where(v_bad > 0.0, -1.0, TBOUND * TBOUND / 1.02)
    stat_v[0:1, :] = jnp.broadcast_to(kn2, (1, 128))
    stat_v[1:2, :] = jnp.broadcast_to(lim, (1, 128))
    stat_v[8:16, :] = jnp.zeros((8, 128), f32)
    h2_v[:, 512:640] = jnp.zeros((64, 128), u32)
    set_flag(qn0, 0)

    def late_setup():
        cp_mod2.wait()
        cp_wo.wait()
        wot_v[...] = wo_v[...].T
        for i in range(2):
            m2 = mod_cols((2 + 2 * i) * D, 2 * D)
            modc_v[2 + 2 * i] = m2[0:D] + float(i)
            modc_v[3 + 2 * i] = m2[D:2 * D]
        set_flag(q_block(h1_of(1), 1), 1)

    class Unit:
        def __init__(self, qi, gb, gc, gd, par, y_first=False, drs=DR5):
            self.qi, self.gb, self.gc, self.gd, self.par = qi, gb, gc, gd, par
            self.y_first, self.drs = y_first, drs
            self.o = [None] * 8
            self.carry = None
            self.qrows = {}
            self.never = None

        def score_mm(self, u, r0, r1, after=None):
            q = q_v[self.qi, 16 * u:16 * u + 16, :]
            if after is not None:
                if self.never is None:
                    self.never = (stat_v[8:16, :] > 0.0)[None]
                q = jnp.concatenate([jnp.where(self.never[0], pltpu.bitcast(after, u32), q[0:8]), q[8:16]], axis=0)
            q = jnp.concatenate([q, jnp.zeros((48, TB), u32)], axis=0)
            return jnp.dot(_bf(k_v[r0 // 2:r1 // 2, :]), _bf(q), preferred_element_type=f32)

        def score_put(self, u, r0, s):
            p_v[u, r0:r0 + s.shape[0], :] = jnp.exp2(s)

        def score_vpu(self, u, r0, sa, idx):
            nv = len(idx)
            if u not in self.qrows:
                lo = (u // 4) * 128
                q0 = DH * (u % 4)
                self.qrows[u] = jnp.concatenate(
                    [jnp.broadcast_to(qf_v[self.qi, q0 + d:q0 + d + 1, lo:lo + 128], (8, TB)) for d in range(DH)],
                    axis=1)[None]
            if self.never is None:
                self.never = (stat_v[8:16, :] > 0.0)[None]
            prod = kb_v[r0:r0 + 8 * nv, :].reshape(nv, 8, DH * 128) * self.qrows[u]
            sv = prod[:, :, 0:256]
            for d in range(1, DH // 2):
                sv = sv + prod[:, :, d * 256:(d + 1) * 256]
            sv = sv[:, :, 0:128] + sv[:, :, 128:256]
            runs = []
            for i in idx:
                if runs and runs[-1][1] == i:
                    runs[-1][1] = i + 1
                else:
                    runs.append([i, i + 1])
            pace = jnp.concatenate([sa[8 * a:8 * b] for a, b in runs], axis=0).reshape(nv, 8, TB)
            self.score_put(u, r0, jnp.where(self.never, pace, sv).reshape(8 * nv, TB))

        def pv(self, u, c, last):
            o = self.o
            k0 = c * 128
            oc = jnp.dot(vt_v[u % 4, :, k0:k0 + 128], p_v[u, k0:k0 + 128, :], preferred_element_type=f32)
            o[u] = oc if o[u] is None else o[u] + oc
            if last:
                row24 = lax.broadcasted_iota(i32, (24, TB), 0)
                r1 = 0 if u % 4 == 3 else 23
                on = jnp.where(row24 == r1, 0.0, o[u] * (1.0 / o[u][r1:r1 + 1]))
                base = 16 * u + 8 * (u // 4)
                first = on[0:8] if u % 4 == 0 else on[0:8] + self.carry
                ot_v[self.gb, base:base + 8, :] = first
                if u % 4 == 3:
                    ot_v[self.gb, base + 8:base + 24, :] = on[8:24]
                else:
                    ot_v[self.gb, base + 8:base + 16, :] = on[8:16]
                    self.carry = on[16:24]

        def piece(self, kind, f, j):
            cols = slice(f * 128, (f + 1) * 128)
            par = self.par
            if kind in "gu":
                w_ref = wg_v if kind == "g" else wu_v
                ai = 2 * f + (kind == "u")
                k0, kn_ = KT[j]
                w = w_ref[self.gc, k0:k0 + kn_, cols]
                if kn_ < 128:
                    w = jnp.concatenate([w, jnp.zeros((128 - kn_, 128), bf16)], axis=0)
                    kn_ = 128
                r = jnp.dot(_bf(h2_v[:, k0:k0 + kn_]), w, preferred_element_type=f32)
                if j > 0:
                    r = r + acc_v[par, ai]
                if j < 4:
                    acc_v[par, ai] = r
                elif kind == "g":
                    acc_v[par, ai] = r * pl.reciprocal(1.0 + jnp.exp2(r * (-LOG2E)), approx=True)
                else:
                    a_v[:, cols] = (acc_v[par, ai - 1] * r).astype(bf16)
            else:
                ra, rb = self.drs[j]
                yc = lax.dot_general(wd_v[self.gd, ra:rb, cols], a_v[:, cols], NT, preferred_element_type=f32)
                if self.y_first and f == 0:
                    y_v[ra:rb, :] = yc
                else:
                    y_v[ra:rb, :] += yc

        def ffn_list(self, C, Dn):
            gl = []
            if C:
                gl = [(k, f, j) for j in range(4) for f in range(NFT) for k in "gu"]
                for i in range(NFT + 1):
                    gl += ([("g", i, 4)] if i < NFT else []) + ([("u", i - 1, 4)] if i >= 1 else [])
            dl = []
            nd = len(self.drs)
            if Dn:
                dl = [("d", f, j) for f in range(NFT)
                      for j in (range(nd) if f % 2 == 0 else range(nd - 1, -1, -1))]
            fp = []
            di = 0
            for m, gp in enumerate(gl):
                assert gp[2] < 4 or di == len(dl)
                fp.append(gp)
                while di < len(dl) and (di * 72 <= m * len(dl)
                                        or (di > 0 and dl[di][2] == 4 and dl[di - 1][2] == 4)):
                    fp.append(dl[di])
                    di += 1
            fp += dl[di:]
            return [(self.drs[p[2]][1] - self.drs[p[2]][0] if p[0] == "d" else 128,
                     functools.partial(self.piece, *p), p) for p in fp]

    def body(n, A, B, C, Dn):
        un = Unit(n % 8, (n + 3) % 4, (n + 2) % 4, (n + 1) % 4, n % 2)
        nva, am = 40, 18
        nm = (S - 8 * nva) // am
        order = []
        upto = []
        for i in range(am):
            r0, v0, v1 = 8 * nva + nm * i, nva * i // am, nva * (i + 1) // am
            for c in list(range(r0 // 128, (r0 + nm - 1) // 128 + 1)) + list(range(v0 // 16, (v1 - 1) // 16 + 1)):
                if c not in order:
                    order.append(c)
            upto.append(len(order))
        pq = [(u, c, j == 15) for u in range(8) for j, c in enumerate(order)] if B else []
        npv = 0
        for u in range(8 if A else 0):
            for i in range(am):
                while npv < min(len(pq), 16 * u + upto[i]):
                    un.pv(*pq[npv])
                    npv += 1
                r0, v0, v1 = 8 * nva + nm * i, nva * i // am, nva * (i + 1) // am
                sa = un.score_mm(u, r0, r0 + nm)
                un.score_put(u, r0, sa)
                un.score_vpu(u, 8 * v0, sa, [((2 * j + 1) * (nm // 8)) // (2 * (v1 - v0)) for j in range(v1 - v0)])
        for t in pq[npv:]:
            un.pv(*t)
        for _, thunk, _ in un.ffn_list(C, Dn):
            thunk()

    def e1_wo(b):
        ot = jnp.concatenate([ot_v[g, 0:144, :] for g in range(4)], axis=0).astype(bf16)
        att = _mm4(wot_v, ot)
        x1 = x_v[b].astype(f32) + modc_v[2] * att
        x1_v[b % 2] = x1
        return _stats(x1)

    def e1_wo_piece(b, r, j, st):
        k0, kn_ = KT[j]
        segs = []
        for g in range(4):
            lo, hi = max(k0, 144 * g), min(k0 + kn_, 144 * g + 144)
            if lo < hi:
                segs.append(ot_v[g, lo - 144 * g:hi - 144 * g, :])
        ot = jnp.concatenate(segs, axis=0).astype(bf16)
        rows = slice(144 * r, 144 * r + 144)
        res = jnp.dot(wot_v[rows, k0:k0 + kn_], ot, preferred_element_type=f32)
        if j > 0:
            res = res + x1_v[b % 2, rows, :]
        if j == 4:
            res = x_v[b, rows, :].astype(f32) + modc_v[2, rows, :] * res
            if r == 0:
                st["piv"] = res[0:1]
            st.setdefault("parts", []).append(_stats_part(res, st["piv"]))
        x1_v[b % 2, rows, :] = res

    def e1_q(b, m, r):
        ln2_v[b % 2, 0:1, 0:128] = m
        ln2_v[b % 2, 1:2, 0:128] = r
        qn = q_block(h1_of(jnp.minimum(b + 2, NB - 1)), b % 2)
        for q0 in range(0, D, 144):
            rows = slice(q0, q0 + 144)
            xn = (x1_v[b % 2, rows, :] - ln2_v[b % 2, 0:1, 0:128]) * ln2_v[b % 2, 1:2, 0:128]
            h2t_v[b % 2, rows, :] = (xn * modc_v[4, rows, :] + modc_v[3, rows, :]).astype(bf16)
        return qn

    def e1_tr(b, j):
        k0, kn_ = KT[j]
        h2 = lax.dot_general(_eye(128), h2t_v[b % 2, k0:k0 + kn_, :], NT, preferred_element_type=f32)
        h2n_v[b % 2, :, k0:k0 + kn_] = _u32(h2)

    def h2_switch(b, j):
        k0, kn_ = KT[j]
        h2_v[:, k0:k0 + kn_] = h2n_v[b % 2, :, k0:k0 + kn_]

    def e2_core(b):
        o_v[b % 2] = (x1_v[b % 2] + modc_v[5] * y_v[...]).astype(bf16)

    def superbody(B):
        qb = (B % 2) * 4
        units = [Unit(qb + g, (g + 3) % 4, (g + 2) % 4, (g + 1) % 4, B % 2, y_first=(g == 3), drs=DR2)
                 for g in range(4)]
        l1 = units[1].ffn_list(1, 1)
        for j in range(5):
            i = max(k for k, e in enumerate(l1) if e[2][0] in "gu" and e[2][2] == j)
            l1.insert(i + 1, (0, functools.partial(h2_switch, B - 1, j), ("s", 0, j)))
        l2 = units[2].ffn_list(1, 1)
        last_d = max(i for i, e in enumerate(l2) if e[2][0] == "d")
        l2.insert(last_d + 1, (0, functools.partial(e2_core, B - 2), ("e", 0, 0)))
        fl = units[0].ffn_list(1, 1) + l1 + l2 + units[3].ffn_list(1, 1)
        hist = []

        def take_f():
            rows, thunk, p = fl.pop(0)
            hist.append(p)
            thunk()
            while fl and fl[0][0] == 0:
                _, thunk, p = fl.pop(0)
                assert p[0] != "s" or ("t", 0, p[2]) in hist
                thunk()
            return rows

        RA = 992
        na = RA // 8
        HW, HQ = 7, 9
        wst = {}
        sa = None
        T = [0, 0, 0, 0]

        def other(rows):
            k = min((1, 2, 3), key=lambda m: T[m])
            T[k] += rows

        def anyfree(rows):
            T[T.index(min(T))] += rows
            T.sort()

        for h in range(H):
            un, u = units[h // 8], h % 8
            if h == HW:
                for i, (j, r) in enumerate((j, r) for j in range(5) for r in range(4)):
                    fl.insert(i + 4, (144, functools.partial(e1_wo_piece, B - 1, r, j, wst), ("w", r, j)))
            if h == HQ:
                while len(wst.get("parts", ())) < 4:
                    anyfree(take_f())
                for _ in range(2):
                    anyfree(take_f())
                qn = e1_q(B - 1, *_stats_fin(wst["parts"], wst["piv"]))
                for j in range(5):
                    fl.insert(j, (128, functools.partial(e1_tr, B - 1, j), ("t", 0, j)))
                set_flag(qn, (B - 1) % 2)
                for _ in range(20):
                    anyfree(144)
                for _ in range(2):
                    anyfree(take_f())
            t0 = T[0]
            load = [0.0] * na
            frows = 3 * RA - 384 - (S - RA - KV)
            acc = 0
            for rows, _, p in fl:
                if acc >= frows:
                    break
                w = {"g": 64 if p[2] == 4 else 0, "u": 32 if p[2] == 4 else 0,
                     "w": 150 if p[2] == 4 else 30, "e": 250, "t": 40}.get(p[0], 0)
                i0 = acc * na // frows
                for i in range(i0, min(na, i0 + 16)):
                    load[i] += w / 16.0
                acc += rows
            if h == HQ:
                for i in range(48):
                    load[i] += 10
            if h == H - 1:
                for i in range(na - 12, na):
                    load[i] += 1000
            rate = KV / RA * 36.0
            idx = []
            credit = 18.0
            for i in range(na):
                credit += max(0.0, rate - load[i])
                if credit >= 36.0:
                    credit -= 36.0
                    idx.append(i)
            if len(idx) % 2:
                idx.pop()
            idx = idx[:KV // 8]
            nv = len(idx)
            sa = un.score_mm(u, S - RA, S, sa[RA - 160:RA - 152] if h > 0 else None)
            T[0] += RA
            att = []
            if h == 0:
                att += [("p", 0, c) for c in (8, 0, 9, 1, 10, 5, 2, 11, 6, 12, 3, 7, 13, 4, 14, 15)]
            nb = 6
            b0, b1 = 8 * nv, S - RA
            cuts = [b0 + ((b1 - b0) // 16 * i // nb) * 16 for i in range(nb)] + [b1]
            pvs = [("p", h + 1, c) for c in range(16)] if h < H - 1 else []
            for i in range(nb):
                att += pvs[len(pvs) * i // nb:len(pvs) * (i + 1) // nb] + [("b", cuts[i], cuts[i + 1])]
            arows = sum(24 if a[0] == "p" else a[2] - a[1] for a in att)
            done = 0
            sbs = []
            while att or (fl and min(T[1:]) < T[0]):
                frac = (min(T[1:]) - t0) / (RA * 90 / 100.0)
                if att and (done <= frac * arows or not fl
                            or (h == 0 and att[0][1] == 0 and done <= 2 * frac * arows)):
                    a = att.pop(0)
                    if a[0] == "p":
                        if a[2] == 15 and a[1] >= 8:
                            lim = DH * (a[1] - 7) + 8
                            assert h >= HW and not any(e[2][0] == "w" and KT[e[2][2]][0] < lim for e in fl)
                        units[a[1] // 8].pv(a[1] % 8, a[2], a[2] == 15)
                        rows = 24
                    else:
                        sbs.append((a[1], un.score_mm(u, a[1], a[2])))
                        rows = a[2] - a[1]
                    done += rows
                    other(rows)
                else:
                    other(take_f())
            un.score_put(u, S - RA, sa)
            for r0, sb in sbs:
                un.score_put(u, r0, sb)
            for i in range(0, nv, 16):
                un.score_vpu(u, 8 * i, sa, idx[i:i + 16])
        while fl:
            anyfree(take_f())

    def a_slow(n):
        qi = n % 8

        def head(u, carry):
            w = pl.multiple_of(16 * u, 16)
            s = jnp.dot(_bf(k_v[:, 0:32]), _bf(q_v[qi, pl.ds(w, 16), :]), preferred_element_type=f32)
            p_v[u] = jnp.exp2(s - jnp.max(s, axis=0, keepdims=True))
            return carry

        lax.fori_loop(0, 8, head, 0)

    def step(n, fast):
        @pl.when(n <= 8)
        def _():
            for m, starts in FSTART.items():
                @pl.when(n == m)
                def _():
                    for w, g in starts:
                        f_copy(w, g).start()

            @pl.when(n == 3)
            def _():
                late_setup()

            for m, waits in FWAIT.items():
                @pl.when(n == m)
                def _():
                    for w, g in waits:
                        f_copy(w, g).wait()

        @pl.when(fast)
        def _():
            body(n, 1, 1, 0, 0)

        @pl.when(jnp.logical_not(fast))
        def _():
            @pl.when(jnp.logical_and(n >= 1, n <= 64))
            def _():
                body(n, 0, 1, 0, 0)

            @pl.when(n < 64)
            def _():
                a_slow(n)

        @pl.when(jnp.logical_and(n >= 7, n <= 69))
        def _():
            body(n, 0, 0, 1, 1)

        @pl.when(n == 70)
        def _():
            body(n, 0, 0, 0, 1)

        @pl.when(n == 6)
        def _():
            body(n, 0, 0, 1, 0)
            y_v[...] = jnp.zeros(y_v.shape, f32)

        @pl.when(jnp.logical_and(n % 4 == 0, jnp.logical_and(n >= 4, n <= 64)))
        def _():
            b = n // 4 - 1
            set_flag(e1_q(b, *e1_wo(b)), b % 2)
            for j in range(5):
                e1_tr(b, j)

        @pl.when(jnp.logical_and(n % 4 == 1, jnp.logical_and(n >= 5, n <= 65)))
        def _():
            for j in range(5):
                h2_switch(n // 4 - 1, j)

        @pl.when(jnp.logical_and(n % 4 == 2, n >= 10))
        def _():
            e2_core(n // 4 - 2)
            y_v[...] = jnp.zeros(y_v.shape, f32)

    def block(B, carry):
        fast = jnp.logical_and(B < NB, flag_s[B % 2] == 1)
        sup = jnp.logical_and(fast, B >= 2)

        @pl.when(B >= 4)
        def _():
            o_copy(B - 4, B % 2).wait()

        @pl.when(B == 2)
        def _():
            for w, g in FWAIT2:
                f_copy(w, g).wait()

        @pl.when(sup)
        def _():
            superbody(B)

        @pl.when(jnp.logical_not(sup))
        def _():
            def inner(g, c2):
                step(4 * B + g, fast)
                return c2

            lax.fori_loop(0, 4, inner, 0)

        @pl.when(B >= 2)
        def _():
            o_copy(B - 2, B % 2).start()

        return carry

    lax.fori_loop(0, NB + 2, block, 0)
    o_copy(NB - 2, 0).wait()
    o_copy(NB - 1, 1).wait()


@jax.jit
def pallas_adaLN_cond__grouped_kv_mqa__swiglu_ffn__prompt_kernel(
        A_x, A_wq, A_wk, A_wv, A_wo, B_x, B_w_gate, B_w_up, B_w_down, c, w_mod):
    hb = pl.BlockSpec(memory_space=pl.ANY)
    out = pl.pallas_call(
        _kernel,
        in_specs=[hb] * 10,
        out_specs=hb,
        out_shape=jax.ShapeDtypeStruct((D, S), bf16),
        scratch_shapes=[
            pltpu.VMEM((NB, D, TB), bf16),
            pltpu.VMEM((D, 6 * D), bf16),
            pltpu.VMEM((D, D), bf16),
            pltpu.VMEM((D, D), bf16),
            pltpu.VMEM((D, D), bf16),
            pltpu.VMEM((D, D), bf16),
            pltpu.VMEM((64, D), bf16),
            pltpu.VMEM((6, D, 128), f32),
            pltpu.VMEM((8, 128, 128), u32),
            pltpu.VMEM((8, 80, 256), f32),
            pltpu.VMEM((S // 2, 128), u32),
            pltpu.VMEM((KV, DH * 128), f32),
            pltpu.VMEM((4, 24, S), f32),
            pltpu.VMEM((8, S, TB), f32),
            pltpu.VMEM((4, 160, TB), f32),
            pltpu.VMEM((64, 640), u32),
            pltpu.VMEM((2, 64, 640), u32),
            pltpu.VMEM((2, D, TB), bf16),
            pltpu.VMEM((NB, 16, 256), f32),
            pltpu.VMEM((2, 16, 256), f32),
            pltpu.VMEM((TB, 1280), bf16),
            pltpu.VMEM((2, 2 * NFT, TB, 128), f32),
            pltpu.VMEM((D, TB), f32),
            pltpu.VMEM((2, D, TB), f32),
            pltpu.VMEM((2, D, TB), bf16),
            pltpu.VMEM((4, D, FG), bf16),
            pltpu.VMEM((4, D, FG), bf16),
            pltpu.VMEM((4, D, FG), bf16),
            pltpu.VMEM((32, 128), f32),
            pltpu.VMEM((1, D), bf16),
            pltpu.VMEM((DH, D), bf16),
            pltpu.VMEM((DH, D), bf16),
            pltpu.SemaphoreType.DMA((NB,)),
            pltpu.SemaphoreType.DMA((10,)),
            pltpu.SemaphoreType.DMA((12,)),
            pltpu.SemaphoreType.DMA((2,)),
            pltpu.SMEM((2,), i32),
        ],
        compiler_params=pltpu.CompilerParams(vmem_limit_bytes=110 * 1024 * 1024),
    )(c, A_wk.T, A_wv.T, A_x.reshape(S, D).T, A_wq, A_wo, B_w_gate, B_w_up, B_w_down.T, w_mod)
    return out.T.reshape(1, S, D)
```

```python
import functools

import jax
import jax.numpy as jnp
from jax import lax
import jax.experimental.pallas as pl
import jax.experimental.pallas.tpu as pltpu

S, D, H, DH, F = 2048, 576, 32, 18, 4608
TB = 128
NB = S // TB
FG = F // 4
NFT = FG // 128
EPS = 1e-5
LOG2E = 1.4426950408889634
QSCALE = DH ** -0.5 * LOG2E
TBOUND = 60.0
f32, bf16, u32, i32 = jnp.float32, jnp.bfloat16, jnp.uint32, jnp.int32
KT = [(0, 128), (128, 128), (256, 128), (384, 128), (512, 64)]
KV = 640
DR5 = [(0, 128), (128, 256), (256, 384), (384, 512), (512, 576)]
DR2 = [(0, 288), (288, 576)]
NT = (((1,), (1,)), ((), ()))
FSTART = {0: [(0, 0), (1, 0)], 1: [(2, 0), (0, 1), (1, 1)], 2: [(2, 1), (0, 2), (1, 2)],
          3: [(2, 2), (0, 3), (1, 3), (2, 3)]}
FWAIT = {6: [(0, 0), (1, 0)], 7: [(2, 0), (0, 1), (1, 1)]}
FWAIT2 = [(2, 1), (0, 2), (1, 2), (2, 2), (0, 3), (1, 3), (2, 3)]


def _bf(x):
    return pltpu.bitcast(x, bf16)


def _u32(x):
    return pltpu.bitcast(x.astype(bf16), u32)


def _stats_part(x, piv):
    d = (x - piv).reshape(x.shape[0] // 8, 8, TB)
    return jnp.sum(d, axis=0), jnp.sum(d * d, axis=0)


def _stats_fin(parts, piv):
    s1 = sum(p[0] for p in parts[1:]) + parts[0][0]
    s2 = sum(p[1] for p in parts[1:]) + parts[0][1]
    m1 = jnp.sum(s1, axis=0, keepdims=True) * (1.0 / D)
    m2 = jnp.sum(s2, axis=0, keepdims=True) * (1.0 / D)
    var = jnp.maximum(m2 - m1 * m1, 0.0)
    return piv + m1, lax.rsqrt(var + EPS)


def _stats(x):
    piv = x[0:1]
    return _stats_fin([_stats_part(x[r:r + 144], piv) for r in range(0, D, 144)], piv)


def _eye(n):
    return (lax.broadcasted_iota(i32, (n, n), 0) == lax.broadcasted_iota(i32, (n, n), 1)).astype(bf16)


def _mm4(w_ref, rhs):
    return jnp.concatenate([jnp.dot(w_ref[r:r + 144, :], rhs, preferred_element_type=f32)
                            for r in range(0, D, 144)], axis=0)


def _kernel(c_hbm, wkt_hbm, wvt_hbm, xt_hbm, wq_hbm, wo_hbm, wg_hbm, wu_hbm, wdt_hbm, wmod_hbm,
            out_hbm,
            x_v, wmod_v, wq_v, wo_v, wqt_v, wot_v, wkv_v, modc_v, q_v, qf_v, k_v, kb_v, vt_v,
            p_v, ot_v, h2_v, h2n_v, ln_v, ln2_v, a_v, acc_v, y_v, x1_v, o_v, wg_v, wu_v, wd_v, stat_v,
            c_ref, wkt_ref, wvt_ref,
            sem_x, sem_w, sem_f, sem_o, flag_s):
    def x_copy(b):
        return pltpu.make_async_copy(xt_hbm.at[:, pl.ds(b * TB, TB)], x_v.at[b], sem_x.at[b])

    cp_mod1 = pltpu.make_async_copy(wmod_hbm.at[:, pl.ds(0, 2 * D)], wmod_v.at[:, pl.ds(0, 2 * D)], sem_w.at[6])

    def wq_copy(j):
        return pltpu.make_async_copy(wq_hbm.at[pl.ds(j * 144, 144), :], wq_v.at[pl.ds(j * 144, 144), :],
                                     sem_w.at[2 + j])

    cp_mod2 = pltpu.make_async_copy(wmod_hbm.at[:, pl.ds(2 * D, 4 * D)], wmod_v.at[:, pl.ds(2 * D, 4 * D)],
                                    sem_w.at[0])
    cp_wo = pltpu.make_async_copy(wo_hbm, wo_v, sem_w.at[1])

    def f_copy(w, g):
        src, dst = ((wg_hbm, wg_v), (wu_hbm, wu_v), (wdt_hbm, wd_v))[w]
        return pltpu.make_async_copy(src.at[:, pl.ds(g * FG, FG)], dst.at[g], sem_f.at[w * 4 + g])

    def o_copy(b, slot):
        return pltpu.make_async_copy(o_v.at[slot], out_hbm.at[:, pl.ds(pl.multiple_of(b * TB, TB), TB)],
                                     sem_o.at[slot])

    small = [pltpu.make_async_copy(src, dst, sem_w.at[7 + i]) for i, (src, dst) in enumerate(
        [(c_hbm, c_ref), (wkt_hbm, wkt_ref), (wvt_hbm, wvt_ref)])]
    for cp in small:
        cp.start()
    for b in range(4):
        x_copy(b).start()
    cp_mod1.start()
    for cp in small:
        cp.wait()

    c = c_ref[...].astype(f32)
    sc = jnp.broadcast_to((c * jax.nn.sigmoid(c)).astype(bf16), (16, D))
    wkv_v[...] = jnp.zeros(wkv_v.shape, bf16)
    wkv_v[0:DH, :] = wkt_ref[...]
    wkv_v[32:32 + DH, :] = wvt_ref[...]

    def mod_cols(c0, n):
        m = jnp.dot(sc, wmod_v[:, c0:c0 + n], preferred_element_type=f32)[0:1]
        return jnp.broadcast_to(m, (128, n)).T

    def ln1_stats(b):
        m, r = _stats(x_v[b].astype(f32))
        ln_v[b, 0:1, 0:128] = m
        ln_v[b, 1:2, 0:128] = r

    for b in range(4):
        x_copy(b).wait()
    for b in range(4, 8):
        x_copy(b).start()
    for b in range(4):
        ln1_stats(b)
    cp_mod1.wait()
    for b in range(8, NB):
        x_copy(b).start()
    for j in range(4):
        wq_copy(j).start()
    m1 = mod_cols(0, 2 * D)
    modc_v[0] = m1[0:D]
    modc_v[1] = 1.0 + m1[D:2 * D]

    def h1_of(b):
        xn = (x_v[b].astype(f32) - ln_v[b, 0:1, 0:128]) * ln_v[b, 1:2, 0:128]
        return (xn * modc_v[1] + modc_v[0]).astype(bf16)

    def kv_s1(b):
        if b >= 4:
            ln1_stats(b)
        return jnp.dot(wkv_v[...], h1_of(b), preferred_element_type=f32)

    def kv_s2(b, kvt, kn, va):
        row24 = lax.broadcasted_iota(i32, (24, TB), 0)
        ktb = kvt[0:32].astype(bf16)
        kt = ktb.astype(f32)
        kn = jnp.maximum(kn, jnp.sum(kt * kt, axis=0, keepdims=True))
        va = jnp.maximum(va, jnp.abs(kvt[32:64]))
        for v in range(4):
            vt = kvt[32 - 2 * v:56 - 2 * v]
            vt_v[v, :, b * TB:(b + 1) * TB] = jnp.where(row24 == (0 if v == 3 else 23), 1.0, vt)
        kt128 = jnp.concatenate([ktb, jnp.zeros((96, TB), bf16)], axis=0)
        k_v[b * 64:(b + 1) * 64, :] = _u32(lax.dot_general(_eye(128), kt128, NT, preferred_element_type=f32))
        return kn, va

    def kv_s4(b, part):
        c0, c1 = part * 6 * 128, (part + 1) * 6 * 128
        esel = (lax.broadcasted_iota(i32, (32, 6 * 128), 0)
                == lax.shift_right_logical(lax.broadcasted_iota(i32, (32, 6 * 128), 1), 7) + 6 * part).astype(bf16)
        kb_v[b * TB:(b + 1) * TB, c0:c1] = jnp.dot(_bf(k_v[b * 64:(b + 1) * 64, 0:32]), esel,
                                                   preferred_element_type=f32)

    def q_block(h1, slot):
        qt = _mm4(wqt_v, h1) * QSCALE
        qr = qt.astype(bf16).astype(f32)
        z8 = jnp.zeros((8, TB), f32)
        qz = jnp.concatenate([qr, z8], axis=0)
        row8 = lax.broadcasted_iota(i32, (8, TB), 0)
        qn = None
        for g in range(4):
            r0 = 144 * g
            wins = []
            for u in range(8):
                w = qz[r0 + DH * u:r0 + DH * u + 24]
                wins += [w, z8]
                sq = w * w
                t = sq[0:8] + sq[8:16] + jnp.where(row8 < DH - 16, sq[16:24], 0.0)
                t = jnp.sum(t, axis=0, keepdims=True)
                qn = t if qn is None else jnp.maximum(qn, t)
            q_v[slot * 4 + g] = _u32(jnp.concatenate(wins, axis=0))
            qf_v[slot * 4 + g, 0:72, 0:128] = qr[r0:r0 + 72]
            qf_v[slot * 4 + g, 0:72, 128:256] = qr[r0 + 72:r0 + 144]
        return qn

    def set_flag(qn, slot):
        ok = jnp.where(qn * stat_v[0:1, :] <= stat_v[1:2, :], 1.0, 0.0)
        flag_s[slot] = (jnp.min(ok) > 0.5).astype(i32)

    kn = jnp.zeros((1, TB), f32)
    va = jnp.zeros((32, TB), f32)
    kvts = {}
    kbq = [(b, part) for b in range(KV // TB) for part in range(3)]
    for i in range(NB + 5):
        if i in (4, 8, 12):
            for b in range(i, i + 4):
                x_copy(b).wait()
        if i == 12:
            for j in range(4):
                wq_copy(j).wait()
            cp_mod2.start()
            cp_wo.start()
            wqt_v[...] = wq_v[...].T
        if i < NB:
            kvts[i] = kv_s1(i)
        if 0 <= i - 1 < NB:
            kn, va = kv_s2(i - 1, kvts.pop(i - 1), kn, va)
        if i == NB:
            qn0 = q_block(h1_of(0), 0)
        if kbq and kbq[0][0] + 2 <= i:
            kv_s4(*kbq.pop(0))
    assert not kbq
    kn2 = jnp.max(kn, axis=1, keepdims=True)
    vrow = jnp.max(va, axis=1, keepdims=True)
    v_ok = jnp.logical_or(vrow == 0.0, jnp.logical_and(vrow >= 2.0 ** -40, vrow <= 2.0 ** 40))
    v_bad = jnp.max(jnp.where(v_ok, 0.0, 1.0), axis=0, keepdims=True)
    lim = jnp.where(v_bad > 0.0, -1.0, TBOUND * TBOUND / 1.02)
    stat_v[0:1, :] = jnp.broadcast_to(kn2, (1, 128))
    stat_v[1:2, :] = jnp.broadcast_to(lim, (1, 128))
    stat_v[8:16, :] = jnp.zeros((8, 128), f32)
    h2_v[:, 512:640] = jnp.zeros((64, 128), u32)
    set_flag(qn0, 0)

    def late_setup():
        cp_mod2.wait()
        cp_wo.wait()
        wot_v[...] = wo_v[...].T
        for i in range(2):
            m2 = mod_cols((2 + 2 * i) * D, 2 * D)
            modc_v[2 + 2 * i] = m2[0:D] + float(i)
            modc_v[3 + 2 * i] = m2[D:2 * D]
        set_flag(q_block(h1_of(1), 1), 1)

    class Unit:
        def __init__(self, qi, gb, gc, gd, par, y_first=False, drs=DR5, hold_q=False):
            self.hold_q = hold_q
            self.qi, self.gb, self.gc, self.gd, self.par = qi, gb, gc, gd, par
            self.y_first, self.drs = y_first, drs
            self.o = [None] * 8
            self.carry = None
            self.qrows = {}
            self.never = None

        def score_mm(self, u, r0, r1, after=None):
            q = q_v[self.qi, 16 * u:16 * u + 16, :]
            if after is not None:
                if self.never is None:
                    self.never = (stat_v[8:16, :] > 0.0)[None]
                q = jnp.concatenate([jnp.where(self.never[0], pltpu.bitcast(after, u32), q[0:8]), q[8:16]], axis=0)
            q = jnp.concatenate([q, jnp.zeros((48, TB), u32)], axis=0)
            return jnp.dot(_bf(k_v[r0 // 2:r1 // 2, :]), _bf(q), preferred_element_type=f32)

        def score_put(self, u, r0, s):
            p_v[u, r0:r0 + s.shape[0], :] = jnp.exp2(s)

        def score_vpu(self, u, r0, sa, idx):
            nv = len(idx)
            if self.never is None:
                self.never = (stat_v[8:16, :] > 0.0)[None]
            if u not in self.qrows:
                lo = (u // 4) * 128
                q0 = DH * (u % 4)
                rows = [jnp.broadcast_to(qf_v[self.qi, q0 + d:q0 + d + 1, lo:lo + 128], (8, TB)) for d in range(DH)]
                if self.hold_q:
                    rows = [jnp.where(self.never[0], 0.0, r) if d < 14 else r for d, r in enumerate(rows)]
                self.qrows[u] = jnp.concatenate(rows, axis=1)[None]
            prod = kb_v[r0:r0 + 8 * nv, :].reshape(nv, 8, DH * 128) * self.qrows[u]
            sv = prod[:, :, 0:256]
            for d in range(1, DH // 2):
                sv = sv + prod[:, :, d * 256:(d + 1) * 256]
            sv = sv[:, :, 0:128] + sv[:, :, 128:256]
            runs = []
            for i in idx:
                if runs and runs[-1][1] == i:
                    runs[-1][1] = i + 1
                else:
                    runs.append([i, i + 1])
            pace = jnp.concatenate([sa[8 * a:8 * b] for a, b in runs], axis=0).reshape(nv, 8, TB)
            self.score_put(u, r0, jnp.where(self.never, pace, sv).reshape(8 * nv, TB))

        def pv(self, u, c, last):
            o = self.o
            k0 = c * 128
            oc = jnp.dot(vt_v[u % 4, :, k0:k0 + 128], p_v[u, k0:k0 + 128, :], preferred_element_type=f32)
            o[u] = oc if o[u] is None else o[u] + oc
            if last:
                row24 = lax.broadcasted_iota(i32, (24, TB), 0)
                r1 = 0 if u % 4 == 3 else 23
                on = jnp.where(row24 == r1, 0.0, o[u] * (1.0 / o[u][r1:r1 + 1]))
                base = 16 * u + 8 * (u // 4)
                first = on[0:8] if u % 4 == 0 else on[0:8] + self.carry
                ot_v[self.gb, base:base + 8, :] = first
                if u % 4 == 3:
                    ot_v[self.gb, base + 8:base + 24, :] = on[8:24]
                else:
                    ot_v[self.gb, base + 8:base + 16, :] = on[8:16]
                    self.carry = on[16:24]

        def piece(self, kind, f, j):
            cols = slice(f * 128, (f + 1) * 128)
            par = self.par
            if kind in "gu":
                w_ref = wg_v if kind == "g" else wu_v
                ai = 2 * f + (kind == "u")
                k0, kn_ = KT[j]
                w = w_ref[self.gc, k0:k0 + kn_, cols]
                if kn_ < 128:
                    w = jnp.concatenate([w, jnp.zeros((128 - kn_, 128), bf16)], axis=0)
                    kn_ = 128
                r = jnp.dot(_bf(h2_v[:, k0:k0 + kn_]), w, preferred_element_type=f32)
                if j > 0:
                    r = r + acc_v[par, ai]
                if j < 4:
                    acc_v[par, ai] = r
                elif kind == "g":
                    acc_v[par, ai] = r * pl.reciprocal(1.0 + jnp.exp2(r * (-LOG2E)), approx=True)
                else:
                    a_v[:, cols] = (acc_v[par, ai - 1] * r).astype(bf16)
            else:
                ra, rb = self.drs[j]
                yc = lax.dot_general(wd_v[self.gd, ra:rb, cols], a_v[:, cols], NT, preferred_element_type=f32)
                if self.y_first and f == 0:
                    y_v[ra:rb, :] = yc
                else:
                    y_v[ra:rb, :] += yc

        def ffn_list(self, C, Dn):
            gl = []
            if C:
                gl = [(k, f, j) for j in range(4) for f in range(NFT) for k in "gu"]
                for i in range(NFT + 1):
                    gl += ([("g", i, 4)] if i < NFT else []) + ([("u", i - 1, 4)] if i >= 1 else [])
            dl = []
            nd = len(self.drs)
            if Dn:
                dl = [("d", f, j) for f in range(NFT)
                      for j in (range(nd) if f % 2 == 0 else range(nd - 1, -1, -1))]
            fp = []
            di = 0
            for m, gp in enumerate(gl):
                assert gp[2] < 4 or di == len(dl)
                fp.append(gp)
                while di < len(dl) and (di * 72 <= m * len(dl)
                                        or (di > 0 and dl[di][2] == 4 and dl[di - 1][2] == 4)):
                    fp.append(dl[di])
                    di += 1
            fp += dl[di:]
            return [(self.drs[p[2]][1] - self.drs[p[2]][0] if p[0] == "d" else 128,
                     functools.partial(self.piece, *p), p) for p in fp]

    def body(n, A, B, C, Dn):
        un = Unit(n % 8, (n + 3) % 4, (n + 2) % 4, (n + 1) % 4, n % 2)
        nva, am = 40, 18
        nm = (S - 8 * nva) // am
        order = []
        upto = []
        for i in range(am):
            r0, v0, v1 = 8 * nva + nm * i, nva * i // am, nva * (i + 1) // am
            for c in list(range(r0 // 128, (r0 + nm - 1) // 128 + 1)) + list(range(v0 // 16, (v1 - 1) // 16 + 1)):
                if c not in order:
                    order.append(c)
            upto.append(len(order))
        pq = [(u, c, j == 15) for u in range(8) for j, c in enumerate(order)] if B else []
        npv = 0
        for u in range(8 if A else 0):
            for i in range(am):
                while npv < min(len(pq), 16 * u + upto[i]):
                    un.pv(*pq[npv])
                    npv += 1
                r0, v0, v1 = 8 * nva + nm * i, nva * i // am, nva * (i + 1) // am
                sa = un.score_mm(u, r0, r0 + nm)
                un.score_put(u, r0, sa)
                un.score_vpu(u, 8 * v0, sa, [((2 * j + 1) * (nm // 8)) // (2 * (v1 - v0)) for j in range(v1 - v0)])
        for t in pq[npv:]:
            un.pv(*t)
        for _, thunk, _ in un.ffn_list(C, Dn):
            thunk()

    def e1_wo(b):
        ot = jnp.concatenate([ot_v[g, 0:144, :] for g in range(4)], axis=0).astype(bf16)
        att = _mm4(wot_v, ot)
        x1 = x_v[b].astype(f32) + modc_v[2] * att
        x1_v[b % 2] = x1
        return _stats(x1)

    def e1_wo_piece(b, r, j, st):
        k0, kn_ = KT[j]
        segs = []
        for g in range(4):
            lo, hi = max(k0, 144 * g), min(k0 + kn_, 144 * g + 144)
            if lo < hi:
                segs.append(ot_v[g, lo - 144 * g:hi - 144 * g, :])
        ot = jnp.concatenate(segs, axis=0).astype(bf16)
        rows = slice(144 * r, 144 * r + 144)
        res = jnp.dot(wot_v[rows, k0:k0 + kn_], ot, preferred_element_type=f32)
        if j > 0:
            res = res + x1_v[b % 2, rows, :]
        if j == 4:
            res = x_v[b, rows, :].astype(f32) + modc_v[2, rows, :] * res
            if r == 0:
                st["piv"] = res[0:1]
            st.setdefault("parts", []).append(_stats_part(res, st["piv"]))
        x1_v[b % 2, rows, :] = res

    def e1_q(b, m, r):
        ln2_v[b % 2, 0:1, 0:128] = m
        ln2_v[b % 2, 1:2, 0:128] = r
        qn = q_block(h1_of(jnp.minimum(b + 2, NB - 1)), b % 2)
        for k0, kn_ in KT:
            rows = slice(k0, k0 + kn_)
            xn = (x1_v[b % 2, rows, :] - ln2_v[b % 2, 0:1, 0:128]) * ln2_v[b % 2, 1:2, 0:128]
            h2t = xn * modc_v[4, rows, :] + modc_v[3, rows, :]
            if kn_ < 128:
                h2t = jnp.concatenate([h2t, jnp.zeros((128 - kn_, TB), f32)], axis=0)
            h2n_v[b % 2, :, k0:k0 + 128] = _u32(h2t.T)
        return qn

    def h2_switch(b, j):
        k0, kn_ = KT[j]
        h2_v[:, k0:k0 + kn_] = h2n_v[b % 2, :, k0:k0 + kn_]

    def e2_core(b):
        o_v[b % 2] = (x1_v[b % 2] + modc_v[5] * y_v[...]).astype(bf16)

    def superbody(B):
        qb = (B % 2) * 4
        units = [Unit(qb + g, (g + 3) % 4, (g + 2) % 4, (g + 1) % 4, B % 2, y_first=(g == 3), drs=DR2,
                      hold_q=True)
                 for g in range(4)]
        l1 = units[1].ffn_list(1, 1)
        for j in range(5):
            i = max(k for k, e in enumerate(l1) if e[2][0] in "gu" and e[2][2] == j)
            l1.insert(i + 1, (0, functools.partial(h2_switch, B - 1, j), ("s", 0, j)))
        l2 = units[2].ffn_list(1, 1)
        last_d = max(i for i, e in enumerate(l2) if e[2][0] == "d")
        l2.insert(last_d + 1, (0, functools.partial(e2_core, B - 2), ("e", 0, 0)))
        fl = units[0].ffn_list(1, 1) + l1 + l2 + units[3].ffn_list(1, 1)

        def take_f():
            rows, thunk, _ = fl.pop(0)
            thunk()
            while fl and fl[0][0] == 0:
                _, thunk, p = fl.pop(0)
                assert p[0] != "s" or "h2" in wst
                thunk()
            return rows

        RA = 992
        na = RA // 8
        NVR = 82
        HW, HQ = 7, 9
        wst = {}
        sa = None
        T = [0, 0, 0, 0]

        def other(rows):
            k = min((1, 2, 3), key=lambda m: T[m])
            T[k] += rows

        def anyfree(rows):
            T[T.index(min(T))] += rows
            T.sort()

        for h in range(H):
            un, u = units[h // 8], h % 8
            if h == HW:
                for i, (j, r) in enumerate((j, r) for j in range(5) for r in range(4)):
                    fl.insert(i + 8, (144, functools.partial(e1_wo_piece, B - 1, r, j, wst), ("w", r, j)))
            if h == HQ:
                while len(wst.get("parts", ())) < 4:
                    anyfree(take_f())
                anyfree(take_f())
                qn = e1_q(B - 1, *_stats_fin(wst["parts"], wst["piv"]))
                wst["h2"] = True
                set_flag(qn, (B - 1) % 2)
                for _ in range(20):
                    anyfree(144)
                for _ in range(3):
                    anyfree(take_f())
            t0 = T[0]
            load = [0.0] * na
            frows = 3 * RA - 384 - (S - RA - 8 * NVR)
            acc = 0
            for rows, _, p in fl:
                if acc >= frows:
                    break
                w = {"g": 72 if p[2] == 4 else 0, "u": 32 if p[2] == 4 else 0,
                     "w": 150 if p[2] == 4 else 30, "e": 250}.get(p[0], 0)
                i0 = acc * na // frows
                for i in range(i0, min(na, i0 + 16)):
                    load[i] += w / 16.0
                acc += rows
            if h == HQ:
                for i in range(48):
                    load[i] += 12
            if h == H - 1:
                for i in range(na - 12, na):
                    load[i] += 1000
            if h == HQ - 1:
                for i in range(na - 16, na):
                    load[i] += 1000
            rate = NVR / na * 36.0
            idx = []
            credit = 18.0
            for i in range(na):
                credit += max(0.0, rate - load[i])
                if credit >= 36.0:
                    credit -= 36.0
                    idx.append(i)
            if len(idx) % 2:
                idx.pop()
            idx = idx[:KV // 8]
            nv = len(idx)
            sa = un.score_mm(u, S - RA, S, sa[RA - 176:RA - 168] if h > 0 else None)
            T[0] += RA
            att = []
            if h == 0:
                att += [("p", 0, c) for c in (8, 0, 9, 1, 10, 5, 2, 11, 6, 12, 3, 7, 13, 4, 14, 15)]
            nb = 6
            b0, b1 = 8 * nv, S - RA
            cuts = [b0 + ((b1 - b0) // 16 * i // nb) * 16 for i in range(nb)] + [b1]
            pvs = [("p", h + 1, c) for c in range(16)] if h < H - 1 else []
            for i in range(nb):
                att += pvs[len(pvs) * i // nb:len(pvs) * (i + 1) // nb] + [("b", cuts[i], cuts[i + 1])]
            arows = sum(24 if a[0] == "p" else a[2] - a[1] for a in att)
            done = 0
            sbs = []
            while att or (fl and min(T[1:]) < T[0]):
                frac = (min(T[1:]) - t0) / (RA * 94 / 100.0)
                if att and (done <= frac * arows or not fl
                            or (h == 0 and att[0][1] == 0 and done <= 2 * frac * arows)):
                    a = att.pop(0)
                    if a[0] == "p":
                        if a[2] == 15 and a[1] >= 8:
                            lim = DH * (a[1] - 7) + 8
                            assert h >= HW and not any(e[2][0] == "w" and KT[e[2][2]][0] < lim for e in fl)
                        units[a[1] // 8].pv(a[1] % 8, a[2], a[2] == 15)
                        rows = 24
                    else:
                        sbs.append((a[1], un.score_mm(u, a[1], a[2])))
                        rows = a[2] - a[1]
                    done += rows
                    other(rows)
                else:
                    other(take_f())
            un.score_put(u, S - RA, sa)
            for r0, sb in sbs:
                un.score_put(u, r0, sb)
            for i in range(0, nv, 16):
                un.score_vpu(u, 8 * i, sa, idx[i:i + 16])
        while fl:
            anyfree(take_f())

    def a_slow(n):
        qi = n % 8

        def head(u, carry):
            w = pl.multiple_of(16 * u, 16)
            s = jnp.dot(_bf(k_v[:, 0:32]), _bf(q_v[qi, pl.ds(w, 16), :]), preferred_element_type=f32)
            p_v[u] = jnp.exp2(s - jnp.max(s, axis=0, keepdims=True))
            return carry

        lax.fori_loop(0, 8, head, 0)

    def step(n, fast):
        @pl.when(n <= 8)
        def _():
            for m, starts in FSTART.items():
                @pl.when(n == m)
                def _():
                    for w, g in starts:
                        f_copy(w, g).start()

            @pl.when(n == 3)
            def _():
                late_setup()

            for m, waits in FWAIT.items():
                @pl.when(n == m)
                def _():
                    for w, g in waits:
                        f_copy(w, g).wait()

        @pl.when(fast)
        def _():
            body(n, 1, 1, 0, 0)

        @pl.when(jnp.logical_not(fast))
        def _():
            @pl.when(jnp.logical_and(n >= 1, n <= 64))
            def _():
                body(n, 0, 1, 0, 0)

            @pl.when(n < 64)
            def _():
                a_slow(n)

        @pl.when(jnp.logical_and(n >= 7, n <= 69))
        def _():
            body(n, 0, 0, 1, 1)

        @pl.when(n == 70)
        def _():
            body(n, 0, 0, 0, 1)

        @pl.when(n == 6)
        def _():
            body(n, 0, 0, 1, 0)
            y_v[...] = jnp.zeros(y_v.shape, f32)

        @pl.when(jnp.logical_and(n % 4 == 0, jnp.logical_and(n >= 4, n <= 64)))
        def _():
            b = n // 4 - 1
            set_flag(e1_q(b, *e1_wo(b)), b % 2)

        @pl.when(jnp.logical_and(n % 4 == 1, jnp.logical_and(n >= 5, n <= 65)))
        def _():
            for j in range(5):
                h2_switch(n // 4 - 1, j)

        @pl.when(jnp.logical_and(n % 4 == 2, n >= 10))
        def _():
            e2_core(n // 4 - 2)
            y_v[...] = jnp.zeros(y_v.shape, f32)

    def block(B, carry):
        fast = jnp.logical_and(B < NB, flag_s[B % 2] == 1)
        sup = jnp.logical_and(fast, B >= 2)

        @pl.when(B >= 4)
        def _():
            o_copy(B - 4, B % 2).wait()

        @pl.when(B == 2)
        def _():
            for w, g in FWAIT2:
                f_copy(w, g).wait()

        @pl.when(sup)
        def _():
            superbody(B)

        @pl.when(jnp.logical_not(sup))
        def _():
            def inner(g, c2):
                step(4 * B + g, fast)
                return c2

            lax.fori_loop(0, 4, inner, 0)

        @pl.when(B >= 2)
        def _():
            o_copy(B - 2, B % 2).start()

        return carry

    lax.fori_loop(0, NB + 2, block, 0)
    o_copy(NB - 2, 0).wait()
    o_copy(NB - 1, 1).wait()


@jax.jit
def pallas_adaLN_cond__grouped_kv_mqa__swiglu_ffn__prompt_kernel(
        A_x, A_wq, A_wk, A_wv, A_wo, B_x, B_w_gate, B_w_up, B_w_down, c, w_mod):
    hb = pl.BlockSpec(memory_space=pl.ANY)
    out = pl.pallas_call(
        _kernel,
        in_specs=[hb] * 10,
        out_specs=hb,
        out_shape=jax.ShapeDtypeStruct((D, S), bf16),
        scratch_shapes=[
            pltpu.VMEM((NB, D, TB), bf16),
            pltpu.VMEM((D, 6 * D), bf16),
            pltpu.VMEM((D, D), bf16),
            pltpu.VMEM((D, D), bf16),
            pltpu.VMEM((D, D), bf16),
            pltpu.VMEM((D, D), bf16),
            pltpu.VMEM((64, D), bf16),
            pltpu.VMEM((6, D, 128), f32),
            pltpu.VMEM((8, 128, 128), u32),
            pltpu.VMEM((8, 80, 256), f32),
            pltpu.VMEM((S // 2, 128), u32),
            pltpu.VMEM((KV, DH * 128), f32),
            pltpu.VMEM((4, 24, S), f32),
            pltpu.VMEM((8, S, TB), f32),
            pltpu.VMEM((4, 160, TB), f32),
            pltpu.VMEM((64, 640), u32),
            pltpu.VMEM((2, 64, 640), u32),
            pltpu.VMEM((NB, 16, 256), f32),
            pltpu.VMEM((2, 16, 256), f32),
            pltpu.VMEM((TB, 1280), bf16),
            pltpu.VMEM((2, 2 * NFT, TB, 128), f32),
            pltpu.VMEM((D, TB), f32),
            pltpu.VMEM((2, D, TB), f32),
            pltpu.VMEM((2, D, TB), bf16),
            pltpu.VMEM((4, D, FG), bf16),
            pltpu.VMEM((4, D, FG), bf16),
            pltpu.VMEM((4, D, FG), bf16),
            pltpu.VMEM((32, 128), f32),
            pltpu.VMEM((1, D), bf16),
            pltpu.VMEM((DH, D), bf16),
            pltpu.VMEM((DH, D), bf16),
            pltpu.SemaphoreType.DMA((NB,)),
            pltpu.SemaphoreType.DMA((10,)),
            pltpu.SemaphoreType.DMA((12,)),
            pltpu.SemaphoreType.DMA((2,)),
            pltpu.SMEM((2,), i32),
        ],
        compiler_params=pltpu.CompilerParams(vmem_limit_bytes=110 * 1024 * 1024),
    )(c, A_wk.T, A_wv.T, A_x.reshape(S, D).T, A_wq, A_wo, B_w_gate, B_w_up, B_w_down.T, w_mod)
    return out.T.reshape(1, S, D)
```
